```python
import jax
import jax.numpy as jnp

def _softmax(x, axis=-1):
    return jax.nn.softmax(x, axis=axis)

def _gelu(x):
    return jax.nn.gelu(x, approximate=True)

def _silu(x):
    return jax.nn.silu(x)

def _sigmoid(x):
    return jax.nn.sigmoid(x)

def _layernorm(x, axis=-1, eps=1e-05):
    m = jnp.mean(x, axis=axis, keepdims=True)
    v = jnp.var(x, axis=axis, keepdims=True)
    return (x - m) / jnp.sqrt(v + eps)

def _scatter_add(tgt, idx, src, axis=0):
    return tgt.at[idx].add(src)

def _segment_sum(src, seg, n):
    return jax.ops.segment_sum(src, seg, n)

class _Rng:

    def __init__(self, key):
        self._k = key

    def _next(self):
        self._k, sub = jax.random.split(self._k)
        return sub

    def normal(self, shape):
        return jax.random.normal(self._next(), shape, dtype=jnp.bfloat16)

    def randint(self, lo, hi, shape):
        return jax.random.randint(self._next(), shape, lo, hi, dtype=jnp.int32)

    def uniform(self, shape, lo=0.0, hi=1.0):
        return jax.random.uniform(self._next(), shape, jnp.bfloat16, lo, hi)

    def permutation(self, n):
        return jax.random.permutation(self._next(), n)
kernel_name = 'adaLN_cond__mha_block_cached__moe_arch_mod__prompt'

def setup_inputs():
    _rng = _Rng(jax.random.key(int.from_bytes(__import__("os").urandom(4), "little")))
    _w = lambda a: (lambda t: t.astype(jnp.bfloat16) if jnp.issubdtype(t.dtype, jnp.floating) else t)(jnp.asarray(a))

    def _A_setup():
        B, Sq, D = (1, 2048, 1024)
        H, Sk, Dh = (32, 2048, 128)
        return {'x': _w((lambda *s: _rng.normal(s) * 0.05)(B, Sq, D)), 'k_cache': _w((lambda *s: _rng.normal(s) * 0.05)(B, H, Sk, Dh)), 'v_cache': _w((lambda *s: _rng.normal(s) * 0.05)(B, H, Sk, Dh)), 'wq': _w((lambda *s: _rng.normal(s) * 0.05)(D, H * Dh) * D ** (-0.5)), 'wo': _w((lambda *s: _rng.normal(s) * 0.05)(H * Dh, D) * (H * Dh) ** (-0.5))}
    _A_in = _A_setup()

    def _B_setup():
        B, S, D, F, C = (1, 2048, 1024, 3584, 2)
        return {'x': _w((lambda *s: _rng.normal(s) * 0.05)(B, S, D)), 'w_r': _w((lambda *s: _rng.normal(s) * 0.05)(D)), 'w_gate': _w((lambda *s: _rng.normal(s) * 0.05)(D, F)), 'w_up': _w((lambda *s: _rng.normal(s) * 0.05)(D, F)), 'w_down': _w((lambda *s: _rng.normal(s) * 0.05)(F, D))}
    _B_in = _B_setup()
    return {'A_x': _A_in['x'], 'A_k_cache': _A_in['k_cache'], 'A_v_cache': _A_in['v_cache'], 'A_wq': _A_in['wq'], 'A_wo': _A_in['wo'], 'B_x': _B_in['x'], 'B_w_r': _B_in['w_r'], 'B_w_gate': _B_in['w_gate'], 'B_w_up': _B_in['w_up'], 'B_w_down': _B_in['w_down'], 'c': _w((lambda *s: _rng.normal(s) * 0.05)(1, 1024)), 'w_mod': _w((lambda *s: _rng.normal(s) * 0.05)(1024, 6 * 1024) * 1024 ** (-0.5))}

def reference(A_x, A_k_cache, A_v_cache, A_wq, A_wo, B_x, B_w_r, B_w_gate, B_w_up, B_w_down, c, w_mod):

    def _A_ref(x, k_cache, v_cache, wq, wo):
        B, Sq, D = x.shape
        H, Dh = (32, 128)
        q = (lambda x, *d: x.transpose(*d))((x @ wq).reshape(B, Sq, H, Dh), 0, 2, 1, 3)
        scores = jnp.einsum('bhqd,bhkd->bhqk', q, k_cache) * Dh ** (-0.5)
        p = _softmax(scores, axis=-1)
        o = jnp.einsum('bhqk,bhkd->bhqd', p, v_cache)
        return (lambda x, *d: x.transpose(*d))(o, 0, 2, 1, 3).reshape(B, Sq, H * Dh) @ wo

    def _B_ref(x, w_r, w_gate, w_up, w_down):
        B, S, D = x.shape
        C = 2
        r = x @ w_r
        idx = jnp.argsort(-r, axis=-1)[:, :C]
        idx_e = jnp.repeat(idx.reshape(B, C, 1), D, axis=2)
        x_sel = jnp.take_along_axis(x, idx_e, axis=1)
        g = _silu(x_sel @ w_gate)
        u = x_sel @ w_up
        y = g * u @ w_down
        r_sel = _sigmoid(jnp.take_along_axis(r, idx, axis=1))
        y = y * r_sel.reshape(B, C, 1)
        b_off = (jnp.arange(B) * S).reshape(B, 1)
        flat_idx = (idx + b_off).reshape(B * C)
        zero = (x * 0.0).reshape(B * S, D)
        upd = _scatter_add(zero, flat_idx, y.reshape(B * C, D), axis=0)
        return x + upd.reshape(B, S, D)
    x = A_x
    mod = (_silu(c) @ w_mod).reshape(c.shape[0], 6, 1, -1)
    sa, ca, ga, sb, cb, gb = (mod[:, 0].copy(), mod[:, 1].copy(), mod[:, 2].copy(), mod[:, 3].copy(), mod[:, 4].copy(), mod[:, 5].copy())
    h = _layernorm(x, axis=-1) * (1 + ca) + sa
    x = x + ga * _A_ref(h, A_k_cache, A_v_cache, A_wq, A_wo)
    h = _layernorm(x, axis=-1) * (1 + cb) + sb
    x = x + gb * _B_ref(h, B_w_r, B_w_gate, B_w_up, B_w_down)
    return x
```

```python
import jax
import jax.numpy as jnp
import jax.experimental.pallas as pl
import jax.experimental.pallas.tpu as pltpu
from jax import lax

BF = jnp.bfloat16
F32 = jnp.float32
I32 = jnp.int32

S = 2048
D = 1024
H = 32
DH = 128
FF = 3584
NP = D // 128
NF = FF // 128
EPS = 1e-5
QSCALE = float(DH ** -0.5 * 1.4426950408889634)
L_LO = 2.0 ** -30
L_HI = 2.0 ** 40

RB = 256
NRB = S // RB
BQ = 256
G0 = 4

NN = (((1,), (0,)), ((), ()))
NT = (((1,), (1,)), ((), ()))


def _b16(x):
    return pltpu.bitcast(x, BF)


def _i32(x):
    return pltpu.bitcast(x, I32)


def _rbf(x):
    return x.astype(BF).astype(F32)


def _dot(a, b, dims=NN):
    return lax.dot_general(a, b, dims, preferred_element_type=F32)


def _ld(ref32, lead, r0, n):
    return _b16(ref32[lead, pl.ds(r0 // 2, n // 2), :])


def _layernorm(x):
    m = _rbf(jnp.mean(x, axis=-1, keepdims=True))
    d = x - m
    mf = jnp.mean(x, axis=-1, keepdims=True)
    df = x - mf
    v = _rbf(jnp.mean(df * df, axis=-1, keepdims=True))
    s = _rbf(jnp.sqrt(_rbf(v + EPS)))
    return d * (1.0 / s)


def _kernel(x_hbm, k_hbm, v_hbm, wq_hbm, wo_hbm, wr_ref, wg_hbm, wu_hbm, wd_hbm, c_ref, wm_hbm,
            out_hbm,
            x_s, out_s, h_s, q_s, wq_s, wo_s, wg_s, wu_s, wd_s, wm_s, k_s, v_s, mod_s, t_s,
            sem_x, sem_wq, sem_wo, sem_g, sem_u, sem_d, sem_m, sem_k, sem_v, sem_o):
    wq32 = wq_s.bitcast(I32)
    wo32 = wo_s.bitcast(I32)
    wg32 = wg_s.bitcast(I32)
    wu32 = wu_s.bitcast(I32)
    wd32 = wd_s.bitcast(I32)
    wm32 = wm_s.bitcast(I32)
    k32 = k_s.bitcast(I32)
    v32 = v_s.bitcast(I32)

    def mo(i, m):
        return i if isinstance(i, int) else pl.multiple_of(i, m)

    def col(j):
        return pl.ds(mo(j * 128, 128), 128)

    def cp_x(rb):
        return pltpu.make_async_copy(x_hbm.at[pl.ds(rb * RB, RB), :], x_s.at[pl.ds(rb * RB, RB), :], sem_x.at[rb])

    def cp_wq(h):
        return pltpu.make_async_copy(wq_hbm.at[:, col(h)], wq_s.at[h], sem_wq.at[h])

    def cp_wo(j):
        return pltpu.make_async_copy(wo_hbm.at[:, col(j)], wo_s.at[j], sem_wo.at[j])

    def cp_g(j):
        return pltpu.make_async_copy(wg_hbm.at[:, col(j)], wg_s.at[j], sem_g.at[j])

    def cp_u(j):
        return pltpu.make_async_copy(wu_hbm.at[:, col(j)], wu_s.at[j], sem_u.at[j])

    def cp_d(j):
        return pltpu.make_async_copy(wd_hbm.at[:, col(j)], wd_s.at[j], sem_d.at[j])

    def cp_m(j):
        return pltpu.make_async_copy(wm_hbm.at[:, col(j)], wm_s.at[j], sem_m.at[j])

    def cp_k(h, slot):
        return pltpu.make_async_copy(k_hbm.at[h], k_s.at[slot], sem_k.at[slot])

    def cp_v(h, slot):
        return pltpu.make_async_copy(v_hbm.at[h], v_s.at[slot], sem_v.at[slot])

    def cp_o(r0, n, i):
        return pltpu.make_async_copy(out_s.at[pl.ds(r0, n), :], out_hbm.at[pl.ds(r0, n), :], sem_o.at[i])

    for j in range(NP):
        cp_m(j).start()
        cp_m(NP + j).start()
    cp_x(0).start()
    for h in range(G0):
        cp_wq(h).start()
    for rb in range(1, NRB):
        cp_x(rb).start()
    for h in range(G0, H):
        cp_wq(h).start()
    cp_k(0, 0).start()
    cp_v(0, 0).start()
    for j in range(2 * NP, 6 * NP):
        cp_m(j).start()

    cf = c_ref[...].astype(F32)
    sc = _rbf(cf * _rbf(jax.nn.sigmoid(cf)))
    sc16 = jnp.broadcast_to(sc, (16, D)).astype(BF)

    def mod_panel(j):
        cp_m(j).wait()
        r = _rbf(_dot(sc16, _b16(wm32[j]))[0:8, :])
        return r

    for j in range(NP):
        mod_s[j] = mod_panel(j)
        mod_s[NP + j] = _rbf(1.0 + mod_panel(NP + j))

    def ln1(r0, n):
        x = x_s[pl.ds(r0, n), :].astype(F32)
        y = _layernorm(x)
        for j in range(NP):
            hj = y[:, j * 128:(j + 1) * 128] * mod_s[NP + j, 0:1, :] + mod_s[j, 0:1, :]
            h_s[j, pl.ds(r0 // 2, n // 2), :] = _i32(hj.astype(BF))

    def qproj(h, r0, n):
        a = jnp.concatenate([_ld(h_s, kc, r0, n) for kc in range(NP)], axis=1)
        q = _dot(a, _b16(wq32[h])) * QSCALE
        return q.astype(BF)

    def phase_a(rb, carry):
        r0 = mo(rb * RB, RB)
        cp_x(rb).wait()
        for t in range(RB // 64):
            ln1(mo(r0 + t * 64, 64), 64)
        for h in range(G0):
            q_s[h, pl.ds(mo(r0 // 2, RB // 2), RB // 2), :] = _i32(qproj(h, r0, RB))
        return carry

    for h in range(G0):
        cp_wq(h).wait()
    lax.fori_loop(0, NRB, phase_a, 0)

    def phase_b(g, carry):
        for hh in range(G0):
            h = G0 + g * G0 + hh
            cp_wq(h).wait()
        for hh in range(G0):
            h = G0 + g * G0 + hh
            for rb in range(NRB):
                q_s[h, pl.ds(rb * RB // 2, RB // 2), :] = _i32(qproj(h, rb * RB, RB))
        return carry

    lax.fori_loop(0, H // G0 - 1, phase_b, 0)

    for j in range(2 * NP, 6 * NP):
        r = mod_panel(j)
        if j // NP == 4:
            r = _rbf(1.0 + r)
        mod_s[j] = r

    def attn_head(h, carry):
        lmin, lmax, osum = carry
        slot = h % 2
        cp_k(h, slot).wait()
        cp_v(h, slot).wait()

        @pl.when(h + 1 < H)
        def _():
            cp_k(h + 1, 1 - slot).start()
            cp_v(h + 1, 1 - slot).start()

        @pl.when(h < NF)
        def _():
            cp_g(h).start()
            cp_u(h).start()

        @pl.when(h < NP)
        def _():
            cp_d(h).start()
            cp_wo(h).start()

        k = _b16(k32[slot])
        v = _b16(v32[slot])
        for ci in range(S // BQ):
            q = _ld(q_s, h, ci * BQ, BQ)
            s = _dot(q, k, NT)
            p = jnp.exp2(s)
            l = jnp.sum(p, axis=1, keepdims=True)
            o = _dot(p.astype(BF), v) * (1.0 / l)
            q_s[h, pl.ds(ci * BQ // 2, BQ // 2), :] = _i32(o.astype(BF))
            for t in range(BQ // 8):
                lt = l[t * 8:(t + 1) * 8]
                lmin = jnp.minimum(lmin, lt)
                lmax = jnp.maximum(lmax, lt)
                osum = osum + o[t * 8:(t + 1) * 8]
        return lmin, lmax, osum

    init = (jnp.full((8, 1), 3e38, F32), jnp.zeros((8, 1), F32), jnp.zeros((8, 128), F32))
    lmin, lmax, osum = lax.fori_loop(0, H, attn_head, init)

    lo = jnp.min(lmin)
    hi = jnp.max(lmax)
    fin = jnp.max(jnp.where(jnp.abs(osum) < 3e38, 0.0, 1.0))
    bad = jnp.logical_or(jnp.logical_or(jnp.logical_not(lo >= L_LO), jnp.logical_not(hi <= L_HI)), fin > 0.5)

    @pl.when(bad)
    def _():
        def safe_head(h, carry):
            ck, cv = cp_k(h, 0), cp_v(h, 0)
            ck.start()
            cv.start()
            ck.wait()
            cv.wait()

            def chunk(ci, carry2):
                r0 = mo(ci * 128, 128)
                q = qproj(h, r0, 128)
                s = _dot(q, _b16(k32[0]), NT)
                p = jnp.exp2(s - jnp.max(s, axis=1, keepdims=True))
                l = jnp.sum(p, axis=1, keepdims=True)
                o = _dot(p.astype(BF), _b16(v32[0])) * (1.0 / l)
                q_s[h, pl.ds(mo(ci * 64, 64), 64), :] = _i32(o.astype(BF))
                return carry2

            lax.fori_loop(0, S // 128, chunk, 0)
            return carry

        lax.fori_loop(0, H, safe_head, 0)

    for j in range(NP):
        cp_wo(j).wait()
    wr = wr_ref[...].astype(F32)

    def oproj(rb, carry):
        m1, i1, m2, i2 = carry
        r0 = mo(rb * RB, RB)
        a = jnp.concatenate([_ld(q_s, h, r0, RB) for h in range(H)], axis=1)
        for j in range(NP):
            t = _rbf(_rbf(_dot(a, _b16(wo32[j]))) * mod_s[2 * NP + j, 0:1, :])
            t_s[:, j * 128:(j + 1) * 128] = t
        for t in range(RB // 64):
            rr = mo(r0 + t * 64, 64)
            x1 = _rbf(x_s[pl.ds(rr, 64), :].astype(F32) + t_s[pl.ds(t * 64, 64), :])
            x_s[pl.ds(rr, 64), :] = x1.astype(BF)
            y = _layernorm(x1)
            racc = None
            for j in range(NP):
                sl = slice(j * 128, (j + 1) * 128)
                hj = _rbf(y[:, sl] * mod_s[4 * NP + j, 0:1, :] + mod_s[3 * NP + j, 0:1, :])
                h_s[j, pl.ds(rr // 2, 32), :] = _i32(hj.astype(BF))
                out_s[pl.ds(rr, 64), sl] = (x1[:, sl] + mod_s[5 * NP + j, 0:1, :] * hj).astype(BF)
                rp = hj * wr[:, sl]
                racc = rp if racc is None else racc + rp
            r = _rbf(jnp.sum(racc, axis=1, keepdims=True))
            for g in range(8):
                v = r[g * 8:(g + 1) * 8]
                idx = lax.broadcasted_iota(I32, (8, 1), 0) + (rr + g * 8)
                gt1 = v > m1
                gt2 = v > m2
                m2 = jnp.where(gt1, m1, jnp.where(gt2, v, m2))
                i2 = jnp.where(gt1, i1, jnp.where(gt2, idx, i2))
                m1 = jnp.where(gt1, v, m1)
                i1 = jnp.where(gt1, idx, i1)
        cp_o(r0, RB, rb).start()
        return m1, i1, m2, i2

    ninf = jnp.full((8, 1), -jnp.inf, F32)
    sub = lax.broadcasted_iota(I32, (8, 1), 0)
    m1, i1, m2, i2 = lax.fori_loop(0, NRB, oproj, (ninf, sub, ninf, sub + 8))

    big = jnp.int32(1 << 30)
    ra = jnp.max(m1, axis=0, keepdims=True)
    ia = jnp.min(jnp.where(m1 == ra, i1, big), axis=0, keepdims=True)
    win = i1 == ia
    mm = jnp.where(win, m2, m1)
    ii = jnp.where(win, i2, i1)
    rb_ = jnp.max(mm, axis=0, keepdims=True)
    ib = jnp.min(jnp.where(mm == rb_, ii, big), axis=0, keepdims=True)
    sa = jnp.clip(ia[0, 0], 0, S - 1)
    sb = jnp.clip(ib[0, 0], 0, S - 1)

    def grp(si):
        return mo((si // 16) * 16, 16)

    row16 = lax.broadcasted_iota(I32, (16, 128), 0)

    def gather(si):
        g0 = grp(si)
        msk = row16 == (si - g0)
        parts = []
        for j in range(NP):
            hj = _b16(h_s[j, pl.ds(mo(g0 // 2, 8), 8), :]).astype(F32)
            parts.append(jnp.sum(jnp.where(msk, hj, 0.0), axis=0, keepdims=True))
        return jnp.broadcast_to(jnp.concatenate(parts, axis=1), (8, D))

    xs = jnp.concatenate([gather(sa), gather(sb)], axis=0).astype(BF)

    for j in range(NF):
        cp_g(j).wait()
        cp_u(j).wait()
    for j in range(NP):
        cp_d(j).wait()

    hid = []
    for j in range(NF):
        g = _rbf(_dot(xs, _b16(wg32[j])))
        u = _rbf(_dot(xs, _b16(wu32[j])))
        g = _rbf(g * _rbf(jax.nn.sigmoid(g)))
        hid.append((g * u).astype(BF))
    hid = jnp.concatenate(hid, axis=1)
    rs = jnp.concatenate([jnp.broadcast_to(_rbf(jax.nn.sigmoid(ra)), (8, 1)),
                          jnp.broadcast_to(_rbf(jax.nn.sigmoid(rb_)), (8, 1))], axis=0)
    ys = [_rbf(_rbf(_dot(hid, _b16(wd32[j]))) * rs) for j in range(NP)]

    for rb in range(NRB):
        cp_o(rb * RB, RB, rb).wait()

    def patch(si):
        g0 = grp(si)
        m_a = row16 == (sa - g0)
        m_b = row16 == (sb - g0)
        for j in range(NP):
            sl = slice(j * 128, (j + 1) * 128)
            ya = jnp.broadcast_to(ys[j][0:1, :], (16, 128))
            yb = jnp.broadcast_to(ys[j][8:9, :], (16, 128))
            upd = jnp.where(m_a, ya, jnp.where(m_b, yb, 0.0))
            hj = _b16(h_s[j, pl.ds(mo(g0 // 2, 8), 8), :]).astype(F32)
            x1 = x_s[pl.ds(g0, 16), sl].astype(F32)
            out_s[pl.ds(g0, 16), sl] = (x1 + mod_s[5 * NP + j, 0:1, :] * _rbf(hj + upd)).astype(BF)

    patch(sa)
    patch(sb)
    ga_, gb_ = grp(sa), grp(sb)
    ca = cp_o(ga_, 16, 0)
    cb = cp_o(gb_, 16, 1)
    ca.start()

    @pl.when(ga_ != gb_)
    def _():
        cb.start()
        cb.wait()

    ca.wait()


@jax.jit
def pallas_adaLN_cond__mha_block_cached__moe_arch_mod__prompt_kernel(
    A_x: jax.Array,
    A_k_cache: jax.Array,
    A_v_cache: jax.Array,
    A_wq: jax.Array,
    A_wo: jax.Array,
    B_x: jax.Array,
    B_w_r: jax.Array,
    B_w_gate: jax.Array,
    B_w_up: jax.Array,
    B_w_down: jax.Array,
    c: jax.Array,
    w_mod: jax.Array,
):
    del B_x
    hbm = pl.BlockSpec(memory_space=pl.ANY)
    vmem = pl.BlockSpec(memory_space=pltpu.VMEM)
    dma = pltpu.SemaphoreType.DMA
    out = pl.pallas_call(
        _kernel,
        out_shape=jax.ShapeDtypeStruct((S, D), BF),
        in_specs=[hbm, hbm, hbm, hbm, hbm, vmem, hbm, hbm, hbm, vmem, hbm],
        out_specs=hbm,
        scratch_shapes=[
            pltpu.VMEM((S, D), BF),
            pltpu.VMEM((S, D), BF),
            pltpu.VMEM((NP, S // 2, 128), I32),
            pltpu.VMEM((H, S // 2, 128), I32),
            pltpu.VMEM((H, D, 128), BF),
            pltpu.VMEM((NP, H * DH, 128), BF),
            pltpu.VMEM((NF, D, 128), BF),
            pltpu.VMEM((NF, D, 128), BF),
            pltpu.VMEM((NP, FF, 128), BF),
            pltpu.VMEM((6 * NP, D, 128), BF),
            pltpu.VMEM((2, S, DH), BF),
            pltpu.VMEM((2, S, DH), BF),
            pltpu.VMEM((6 * NP, 8, 128), F32),
            pltpu.VMEM((RB, D), F32),
            dma((NRB,)), dma((H,)), dma((NP,)), dma((NF,)), dma((NF,)), dma((NP,)), dma((6 * NP,)),
            dma((2,)), dma((2,)), dma((NRB,)),
        ],
        compiler_params=pltpu.CompilerParams(vmem_limit_bytes=120 * 1024 * 1024),
    )(A_x.reshape(S, D), A_k_cache.reshape(H, S, DH), A_v_cache.reshape(H, S, DH), A_wq, A_wo,
      B_w_r.reshape(1, D), B_w_gate, B_w_up, B_w_down, c, w_mod)
    return out.reshape(1, S, D)
```

```python
import jax
import jax.numpy as jnp
import jax.experimental.pallas as pl
import jax.experimental.pallas.tpu as pltpu
from jax import lax

BF = jnp.bfloat16
F32 = jnp.float32
I32 = jnp.int32

S = 2048
D = 1024
H = 32
DH = 128
FF = 3584
NP = D // 128
NF = FF // 128
EPS = 1e-5
QSCALE = float(DH ** -0.5 * 1.4426950408889634)
L_LO = 2.0 ** -30
L_HI = 2.0 ** 40

XB = 256
NXB = S // XB
R = 64
NSL = S // (2 * R)
P0 = 4
PPI = 2
BQ = 256
HPI = 2
X_STAGES = (0, 128, 512, 1024, 2048)
DPI = 2

NN = (((1,), (0,)), ((), ()))
NT = (((1,), (1,)), ((), ()))


def _b16(x):
    return pltpu.bitcast(x, BF)


def _i32(x):
    return pltpu.bitcast(x, I32)


def _rbf(x):
    return x.astype(BF).astype(F32)


def _dot(a, b, dims=NN):
    return lax.dot_general(a, b, dims, preferred_element_type=F32)


def _unpk(w):
    return (pltpu.unpack_elementwise(w, index=0, packed_dtype=BF, unpacked_dtype=F32),
            pltpu.unpack_elementwise(w, index=1, packed_dtype=BF, unpacked_dtype=F32))


def _pk(even, odd):
    return pltpu.bitcast(pltpu.pack_elementwise([even, odd], packed_dtype=BF), I32)


def _zero_after(v):
    i = pltpu.bitcast(v[0:8, :], I32)
    return lax.shift_right_logical(lax.shift_right_logical(i, 31), 1)


def _tie(x, z):
    if z is None:
        return x
    if x.dtype == I32:
        head = x[0:8] + z
    else:
        head = pltpu.bitcast(pltpu.bitcast(x[0:8], I32) + z, x.dtype)
    return head if x.shape[0] == 8 else jnp.concatenate([head, x[8:]], axis=0)


def _ln_parts(parts, extra=None):
    tot = parts[0]
    for p in parts[1:]:
        tot = tot + p
    m = jnp.sum(tot, axis=1, keepdims=True) * (1.0 / D)
    dfs = [p - m for p in parts]
    sq = dfs[0] * dfs[0]
    for d in dfs[1:]:
        sq = sq + d * d
    v = _rbf(_rbf(jnp.sum(sq, axis=1, keepdims=True) * (1.0 / D)) + EPS)
    rs = lax.rsqrt(v)
    s = _rbf(v * rs)
    return dfs, rs * (2.0 - s * rs)


def _strassen(prod):
    m1 = prod(0)
    m5 = prod(4)
    m4 = prod(3)
    m7 = prod(6)
    c11 = m1 + m4 - m5 + m7
    m3 = prod(2)
    c12 = m3 + m5
    m2 = prod(1)
    c21 = m2 + m4
    m6 = prod(5)
    c22 = m1 - m2 + m3 + m6
    return c11, c12, c21, c22


def _kernel(x_hbm, k_hbm, v_hbm, wq_hbm, wo_hbm, wr_hbm, wg_hbm, wu_hbm, wd_hbm, c_hbm, wm_hbm,
            out_hbm,
            x_s, out_s, lq_s, h_s, q_s, wq_s, wo_s, ro_s, wg_s, wu_s, wd_s, wm_s, k_s, v_s, mod_s,
            t0_s, t1_s, lo0_s, lo1_s, ra_s, rb_s, rc_s, rd_s, re_s, rf_s, c_s, wr_s, ccol_s, cc2_s, pst_s,
            sem_x, sem_wq, sem_wo, sem_mlp, sem_m, sem_k, sem_v, sem_o, sem_s):
    wq32 = wq_s.bitcast(I32)
    wo32 = wo_s.bitcast(I32)
    wg32 = wg_s.bitcast(I32)
    wu32 = wu_s.bitcast(I32)
    wd32 = wd_s.bitcast(I32)
    wm32 = wm_s.bitcast(I32)
    k32 = k_s.bitcast(I32)
    v32 = v_s.bitcast(I32)
    x32 = x_s.bitcast(I32)
    out32 = out_s.bitcast(I32)
    pst32 = pst_s.bitcast(I32)

    def mo(i, m):
        return i if isinstance(i, int) else pl.multiple_of(i, m)

    def col(j):
        return pl.ds(mo(j * 128, 128), 128)

    def cp_x(st, j):
        r0, n = X_STAGES[st], X_STAGES[st + 1] - X_STAGES[st]
        return pltpu.make_async_copy(x_hbm.at[pl.ds(r0, n), col(j)], x_s.at[j, pl.ds(r0, n), :], sem_x.at[st])

    def cp_wq(h, g):
        return pltpu.make_async_copy(wq_hbm.at[:, col(h)], wq_s.at[h], sem_wq.at[g])

    def cp_m(j, g):
        return pltpu.make_async_copy(wm_hbm.at[:, col(j)], wm_s.at[j], sem_m.at[g])

    def m_panel(i):
        return i // 4 + 4 * (i % 4)

    def cp_wo(j):
        return pltpu.make_async_copy(wo_hbm.at[:, col(j)], wo_s.at[j], sem_wo.at[0])

    def cp_w(src, dst, j):
        return pltpu.make_async_copy(src.at[:, col(j)], dst.at[j], sem_mlp.at[0])

    def cp_kv(g, slot):
        return (pltpu.make_async_copy(k_hbm.at[pl.ds(g * HPI, HPI)], k_s.at[slot], sem_k.at[slot]),
                pltpu.make_async_copy(v_hbm.at[pl.ds(g * HPI, HPI)], v_s.at[slot], sem_v.at[slot]))

    def cp_o(r0, n, j, i):
        return pltpu.make_async_copy(out_s.at[j, pl.ds(r0, n), :], out_hbm.at[pl.ds(r0, n), col(j)], sem_o.at[i])

    cp_c = pltpu.make_async_copy(c_hbm, c_s, sem_s.at[0])
    cp_r = pltpu.make_async_copy(wr_hbm, wr_s, sem_s.at[1])
    cp_c.start()

    @pl.loop(0, NP)
    def _(j):
        cp_x(0, j).start()

    @pl.loop(0, 2 * P0)
    def _(h):
        cp_wq(h, 0).start()

    @pl.loop(0, 2 * NP)
    def _(i):
        cp_m(m_panel(i), i // 4).start()

    @pl.loop(0, NP)
    def _(j):
        cp_x(1, j).start()

    def rq_step(p, dst, r0, z=None):
        a, b = 2 * p, 2 * p + 1

        def ld(h, half):
            return _unpk(_tie(wq32[h, pl.ds(half * 256 + r0, 32), :], z))
        b11, b12, b21, b22 = ld(a, 0), ld(b, 0), ld(a, 1), ld(b, 1)
        for i, (u, v, sg) in enumerate(((b11, b22, 1), (b12, b22, -1), (b21, b11, -1), (b11, b12, 1), (b21, b22, 1))):
            dst[i, r0:r0 + 32, :] = _pk(u[0] + v[0], u[1] + v[1]) if sg > 0 else _pk(u[0] - v[0], u[1] - v[1])

    def rq_combos(p, dst):
        for r0 in range(0, 256, 32):
            rq_step(p, dst, r0)

    def lq_store(s, kc, hs, w0, nw):
        ops = [(a11 + a22, a21 + a22, a11, a22, a11 + a12, a21 - a11, a12 - a22) for a11, a12, a21, a22 in hs]
        for i in range(7):
            lq_s[(s * 7 + i) * 4 + kc, w0:w0 + nw, :] = _pk(ops[0][i], ops[1][i])

    def ln1(s, w0, nw, z=None):
        hs = [[], []]
        for half in range(2):
            ww = s * R + half * (R // 2) + w0
            xs = [_unpk(_tie(x32[j, ww:ww + nw, :], z if j == 0 else None)) for j in range(NP)]
            for par in range(2):
                ds, inv = _ln_parts([x_[par] for x_ in xs])
                hs[par].append([(ds[j] * inv) * mod_s[NP + j, 0:1, :] + mod_s[j, 0:1, :] for j in range(NP)])
        for kc in range(4):
            lq_store(s, kc, [(hs[par][0][kc], hs[par][0][kc + 4], hs[par][1][kc], hs[par][1][kc + 4])
                             for par in range(2)], w0, nw)

    def q_slab(p, rsrc, s):
        a, b = 2 * p, 2 * p + 1
        toks = []

        def prod(i):
            lhs = jnp.concatenate([_b16(lq_s[(s * 7 + i) * 4 + kc]) for kc in range(4)], axis=1)
            if i == 1:
                w = wq32[a, 0:256, :]
            elif i == 4:
                w = wq32[b, 256:512, :]
            else:
                w = rsrc[{0: 0, 2: 1, 3: 2, 5: 3, 6: 4}[i]]
            m = _dot(lhs, _b16(w))
            toks.append(m)
            return m

        c11, c12, c21, c22 = _strassen(prod)
        w0 = mo(s * R, R)
        q_s[a, pl.ds(w0, R // 2), :] = _i32(c11.astype(BF))
        q_s[b, pl.ds(w0, R // 2), :] = _i32(c12.astype(BF))
        q_s[a, pl.ds(w0 + R // 2, R // 2), :] = _i32(c21.astype(BF))
        q_s[b, pl.ds(w0 + R // 2, R // 2), :] = _i32(c22.astype(BF))
        return toks

    cp_c.wait()
    for j in range(NP):
        cp_x(0, j).wait()
    cf = c_s[...].astype(F32)
    sc = _rbf(cf * _rbf(jax.nn.sigmoid(cf)))
    sc16 = jnp.broadcast_to(sc, (16, D)).astype(BF)
    for half in range(2):
        xs = [_unpk(x32[j, half * 32:half * 32 + 32, :]) for j in range(NP)]
        for par in range(2):
            ds, inv = _ln_parts([x_[par] for x_ in xs])
            for j in range(NP):
                t0_s[j, par * 64 + half * 32:par * 64 + half * 32 + 32, :] = ds[j] * inv
    scb = jnp.broadcast_to(sc, (128, D))
    for j in range(NP):
        ccol_s[j * 128:(j + 1) * 128, :] = scb[:, j * 128:(j + 1) * 128].T
    ce_s, co_s = cc2_s.at[0], cc2_s.at[1]
    ce_s[...] = ccol_s[pl.ds(0, D // 2, stride=2), :]
    co_s[...] = ccol_s[pl.ds(1, D // 2, stride=2), :]

    for h in range(2 * P0):
        cp_wq(h, 0).wait()
    rsm = (ra_s, rb_s, rc_s, rd_s)
    for p in range(P0):
        rq_combos(p, rsm[p])

    for g in range(4):
        for i in range(4):
            cp_m(m_panel(4 * g + i), g).wait()
        hh = []
        for j in (g, g + 4):
            sa = _rbf(_dot(sc16, _b16(wm32[j]))[0:8, :]) * QSCALE
            ca = _rbf(1.0 + _rbf(_dot(sc16, _b16(wm32[NP + j]))[0:8, :])) * QSCALE
            mod_s[j] = sa
            mod_s[NP + j] = ca
            hh.append(t0_s[j] * ca[0:1, :] + sa[0:1, :])
        lq_store(0, g, [(hh[0][par * 64:par * 64 + 32], hh[1][par * 64:par * 64 + 32],
                         hh[0][par * 64 + 32:par * 64 + 64], hh[1][par * 64 + 32:par * 64 + 64])
                        for par in range(2)], 0, 32)

    NPAIR = H // 2
    NB = (NPAIR - P0) // PPI
    rpp = (re_s, rf_s)
    for s in range(NSL):
        nxt = s + 1
        if nxt < NSL and nxt * 2 * R in X_STAGES:
            st = X_STAGES.index(nxt * 2 * R)
            for j in range(NP):
                cp_x(st, j).wait()
        if s == 0:
            for j in range(NP):
                cp_x(2, j).start()
        if s == 3:
            for j in range(NP):
                cp_x(3, j).start()
            for h in range(2 * P0, 2 * P0 + 2 * PPI + 2):
                cp_wq(h, 1 + (h - 2 * P0) // 2).start()
        if s == 7:
            for h in range(2 * P0 + 2 * PPI + 2, H):
                cp_wq(h, 1 + (h - 2 * P0) // 2).start()
        if s == NSL - 1:
            for h in range(2 * P0, 2 * P0 + 2):
                cp_wq(h, 1).wait()
            cp_r.start()
            for c in cp_kv(0, 0):
                c.start()
            for j in range(NP):
                cp_wo(j).start()
            for j in range(2 * NP, 6 * NP):
                cp_m(j, 4).start()
        toks = []
        for p in range(P0):
            toks += q_slab(p, rsm[p], s)
        if nxt < NSL:
            npc = R // 16
            for i in range(npc):
                ln1(nxt, i * 8, 8, _zero_after(toks[i * len(toks) // npc]))
        else:
            for i in range(8):
                rq_step(P0, rpp[0], i * 32, _zero_after(toks[i * len(toks) // 8]))

    def phase_b(g, carry):
        p0 = P0 + PPI * g
        for u in range(PPI):
            pn = jnp.minimum(p0 + u + 1, NPAIR - 1)

            @pl.when(p0 + u + 1 < NPAIR)
            def _():
                for hh in range(2):
                    cp_wq(2 * pn + hh, 1 + pn - P0).wait()
        for u in range(PPI):
            cur, nxt = rpp[u % 2], rpp[(u + 1) % 2]
            p = p0 + u
            for s in range(NSL):
                toks = q_slab(p, cur, s)
                if 1 <= s <= 8:
                    rq_step(jnp.minimum(p + 1, NPAIR - 1), nxt, (s - 1) * 32, _zero_after(toks[0]))
        return carry

    lax.fori_loop(0, NB, phase_b, 0)

    for j in range(NP):
        cp_wo(j).wait()

    for j in range(2 * NP, 6 * NP):
        cp_m(j, 4).wait()

    def ro_job(g, n, r0, z):
        w0 = mo(g * 64, 64)

        def ld(j, half):
            return _unpk(_tie(wo32[j, pl.ds(w0 + half * 1024 + r0, 16), :], z))
        b11, b12, b21, b22 = ld(n, 0), ld(n + 4, 0), ld(n, 1), ld(n + 4, 1)
        for i, (u, v, sg) in enumerate(((b11, b22, 1), (b12, b22, -1), (b21, b11, -1), (b11, b12, 1), (b21, b22, 1))):
            ro_s[i * 4 + n, pl.ds(w0 + r0, 16), :] = (_pk(u[0] + v[0], u[1] + v[1]) if sg > 0
                                                     else _pk(u[0] - v[0], u[1] - v[1]))

    mst = {}

    def mod_job(j, r, z):
        we, wo_ = _unpk(_tie(wm32[j, r:r + 64, :], z))
        t = we * ce_s[r:r + 64, :] + wo_ * co_s[r:r + 64, :]
        t = jnp.sum(t.reshape(8, 8, 128), axis=0)
        mst['acc'] = t if r == 0 else mst['acc'] + t
        if r == 448:
            v = _rbf(jnp.sum(mst['acc'], axis=0, keepdims=True))
            v = jnp.where(j // NP == 4, _rbf(1.0 + v), v)
            mod_s[j] = jnp.broadcast_to(v, (8, 128))

    def attn_group(g, carry):
        lmin, lmax, osum = carry
        slot = g % 2
        for c in cp_kv(g, slot):
            c.wait()

        @pl.when(g + 1 < H // HPI)
        def _():
            for c in cp_kv(g + 1, 1 - slot):
                c.start()

        @pl.when(g < NF // 2)
        def _():
            for i in range(2):
                cp_w(wg_hbm, wg_s, g * 2 + i).start()
                cp_w(wu_hbm, wu_s, g * 2 + i).start()

        @pl.when(g < NP)
        def _():
            cp_w(wd_hbm, wd_s, g).start()

        ja = [lambda z, n=n, r0=r0: ro_job(g, n, r0, z) for n in range(4) for r0 in range(0, 64, 16)]
        jb = [lambda z, jj=jj, r=r: mod_job(2 * NP + 2 * g + jj, r, z) for jj in range(2) for r in range(0, 512, 64)]
        jobs = [x for pair in zip(ja, jb) for x in pair]
        ntok = HPI * (S // BQ) * 4
        tc = 0
        for hh in range(HPI):
            h = g * HPI + hh
            k = _b16(k32[slot, hh])
            v = _b16(v32[slot, hh])
            for ci in range(S // BQ):
                q = _b16(q_s[h, pl.ds(ci * BQ // 2, BQ // 2), :])
                s = _dot(q, k, NT)
                p = jnp.exp2(s)
                l = jnp.sum(p, axis=1, keepdims=True)
                r0_ = pl.reciprocal(l, approx=True)
                o = _dot(p.astype(BF), v) * (r0_ * (2.0 - l * r0_))
                q_s[h, pl.ds(ci * BQ // 2, BQ // 2), :] = _i32(o.astype(BF))
                for t in range(BQ // 8):
                    lt = l[t * 8:(t + 1) * 8]
                    lmin = jnp.minimum(lmin, lt)
                    lmax = jnp.maximum(lmax, lt)
                    osum = osum + o[t * 8:(t + 1) * 8]
                for tt in range(4):
                    lo_, hi_ = tc * len(jobs) // ntok, (tc + 1) * len(jobs) // ntok
                    if hi_ > lo_:
                        z = _zero_after(s[0:8, tt * 512:tt * 512 + 128])
                        for f in jobs[lo_:hi_]:
                            f(z)
                    tc += 1
        return lmin, lmax, osum

    init = (jnp.full((8, 1), 3e38, F32), jnp.zeros((8, 1), F32), jnp.zeros((8, 128), F32))
    lmin, lmax, osum = lax.fori_loop(0, H // HPI, attn_group, init)

    lo = jnp.min(lmin)
    hi = jnp.max(lmax)
    fin = jnp.max(jnp.where(jnp.abs(osum) < 3e38, 0.0, 1.0))
    bad = jnp.logical_or(jnp.logical_or(jnp.logical_not(lo >= L_LO), jnp.logical_not(hi <= L_HI)), fin > 0.5)

    @pl.when(bad)
    def _():
        def safe_pair(p, carry):
            rq_combos(p, re_s)

            def qs(s, c2):
                q_slab(p, re_s, s)
                return c2

            lax.fori_loop(0, NSL, qs, 0)

            def one_head(hh, c2):
                h = 2 * p + hh
                ck = pltpu.make_async_copy(k_hbm.at[h], k_s.at[0, 0], sem_k.at[0])
                cv = pltpu.make_async_copy(v_hbm.at[h], v_s.at[0, 0], sem_v.at[0])
                ck.start()
                cv.start()
                ck.wait()
                cv.wait()

                def chunk(ci, c3):
                    w0 = mo(ci * 64, 64)
                    q = _b16(q_s[h, pl.ds(w0, 64), :])
                    s = _dot(q, _b16(k32[0, 0]), NT)
                    p_ = jnp.exp2(s - jnp.max(s, axis=1, keepdims=True))
                    l = jnp.sum(p_, axis=1, keepdims=True)
                    o = _dot(p_.astype(BF), _b16(v32[0, 0])) * (1.0 / l)
                    q_s[h, pl.ds(w0, 64), :] = _i32(o.astype(BF))
                    return c3

                lax.fori_loop(0, S // 128, chunk, 0)
                return c2

            lax.fori_loop(0, 2, one_head, 0)
            return carry

        lax.fori_loop(0, NPAIR, safe_pair, 0)

    cp_r.wait()
    for j in range(NF):
        cp_w(wg_hbm, wg_s, j).wait()
        cp_w(wu_hbm, wu_s, j).wait()
    for j in range(NP):
        cp_w(wd_hbm, wd_s, j).wait()
    wr = wr_s[...].astype(F32).reshape(1, D)
    cw = [mod_s[4 * NP + j, 0:1, :] * wr[:, j * 128:(j + 1) * 128] for j in range(NP)]
    sw = mod_s[3 * NP, 0:1, :] * wr[:, 0:128]
    for j in range(1, NP):
        sw = sw + mod_s[3 * NP + j, 0:1, :] * wr[:, j * 128:(j + 1) * 128]
    sw = jnp.sum(sw, axis=1, keepdims=True)

    def lo_combos(w0, r, dst, g, z):
        def ld(h, half):
            return _unpk(_tie(q_s[h, pl.ds(mo(w0 + half * (r // 2), r // 2), r // 2), :], z))
        a11, a12, a21, a22 = ld(g, 0), ld(g + 16, 0), ld(g, 1), ld(g + 16, 1)
        for i, (u, v, sg) in enumerate(((a11, a22, 1), (a21, a22, 1), (a11, a12, 1), (a21, a11, -1), (a12, a22, -1))):
            dst[i * 16 + g, 0:r // 2, :] = (_pk(u[0] + v[0], u[1] + v[1]) if sg > 0
                                            else _pk(u[0] - v[0], u[1] - v[1]))

    def o_slab(w0, r, lsrc, t_ref, side):
        cnt = [0]
        for n in range(4):
            def prod(i):
                if i == 2:
                    pan = [q_s[g, pl.ds(mo(w0, r // 2), r // 2), :] for g in range(16)]
                elif i == 3:
                    pan = [q_s[g + 16, pl.ds(mo(w0 + r // 2, r // 2), r // 2), :] for g in range(16)]
                else:
                    li = {0: 0, 1: 1, 4: 2, 5: 3, 6: 4}[i]
                    pan = [lsrc[li * 16 + g, 0:r // 2, :] for g in range(16)]
                lhs = jnp.concatenate([_b16(a) for a in pan], axis=1)
                if i == 1:
                    w = wo32[n, 0:1024, :]
                elif i == 4:
                    w = wo32[n + 4, 1024:2048, :]
                else:
                    w = ro_s[{0: 0, 2: 1, 3: 2, 5: 3, 6: 4}[i] * 4 + n]
                m = _dot(lhs, _b16(w))
                side(cnt[0], m)
                cnt[0] += 1
                return m
            c11, c12, c21, c22 = _strassen(prod)
            t_ref[n, 0:r, :] = c11
            t_ref[n + 4, 0:r, :] = c12
            t_ref[n, r:2 * r, :] = c21
            t_ref[n + 4, r:2 * r, :] = c22

    state = {}

    def ln2(rr, t_ref, p0, z):
        m1, i1, m2, i2 = state['top']
        ww = mo(rr // 2, 8)
        x1 = [[], []]
        for j in range(NP):
            xe, xo = _unpk(_tie(x32[j, pl.ds(ww, 8), :], z if j == 0 else None))
            ga = mod_s[2 * NP + j]
            e = xe + t_ref[j, pl.ds(p0, 8, stride=2), :] * ga
            o = xo + t_ref[j, pl.ds(p0 + 1, 8, stride=2), :] * ga
            x32[j, pl.ds(ww, 8), :] = _pk(e, o)
            x1[0].append(e)
            x1[1].append(o)
        hs, os_ = [], []
        for par in range(2):
            ds, inv = _ln_parts(x1[par])
            rd = ds[0] * cw[0]
            for j in range(1, NP):
                rd = rd + ds[j] * cw[j]
            v = _rbf(jnp.sum(rd, axis=1, keepdims=True) * inv + sw)
            hj = [(ds[j] * inv) * mod_s[4 * NP + j] + mod_s[3 * NP + j] for j in range(NP)]
            hs.append(hj)
            os_.append([x1[par][j] + mod_s[5 * NP + j] * hj[j] for j in range(NP)])
            idx = 2 * sub + (rr + par)
            gt1 = v > m1
            gt2 = v > m2
            m2 = jnp.where(gt1, m1, jnp.where(gt2, v, m2))
            i2 = jnp.where(gt1, i1, jnp.where(gt2, idx, i2))
            m1 = jnp.where(gt1, v, m1)
            i1 = jnp.where(gt1, idx, i1)
        for j in range(NP):
            h_s[j, pl.ds(ww, 8), :] = _pk(hs[0][j], hs[1][j])
            out32[j, pl.ds(ww, 8), :] = _pk(os_[0][j], os_[1][j])
        state['top'] = (m1, i1, m2, i2)

    ninf = jnp.full((8, 1), -jnp.inf, F32)
    sub = lax.broadcasted_iota(I32, (8, 1), 0)
    state['top'] = (ninf, sub + S, ninf, sub + S + 8)
    tb = (t0_s, t1_s)
    lb = (lo0_s, lo1_s)

    def d_step(row, r, slot, r_next, r_prev):
        jobs = []
        if r_next:
            for g in range(16):
                jobs.append((g * 24 // 16, lambda z, g=g: lo_combos((row + 2 * r) // 2, r_next, lb[1 - slot], g, z)))
        if r_prev:
            npc = 2 * r_prev // 16
            for i in range(npc):
                jobs.append((1 + i * 24 // npc,
                             lambda z, i=i: ln2(row - 2 * r_prev + i * 16, tb[1 - slot], i * 16, z)))

        def side(k, m):
            todo = [f for (slot_, f) in jobs if slot_ == k]
            if todo:
                z = _zero_after(m)
                for f in todo:
                    f(z)

        o_slab(row // 2, r, lb[slot], tb[slot], side)

    for g in range(16):
        lo_combos(0, R, lb[0], g, None)
    d_step(0, R, 0, R, 0)
    ND = (NSL - 2) // DPI
    OB = DPI * 2 * R

    def d_loop(i, top):
        state['top'] = top
        row = mo(2 * R + i * OB, 2 * R)
        for u in range(DPI):
            d_step(row + u * 2 * R, R, (u + 1) % 2, R, R)
        for j in range(NP):
            cp_o(mo(i * OB, OB), OB, j, i).start()
        return state['top']

    state['top'] = lax.fori_loop(0, ND, d_loop, state['top'])
    row = (NSL - 1) * 2 * R
    d_step(row, R // 2, 1, R // 2, R)
    d_step(row + R, R // 2, 0, 0, R // 2)
    for i in range(R // 16):
        ln2(row + R + i * 16, tb[0], i * 16, None)
    out_cps = [cp_o(i * OB, OB, j, i) for i in range(ND) for j in range(NP)]
    for j in range(NP):
        c = cp_o(ND * OB, S - ND * OB, j, ND)
        c.start()
        out_cps.append(c)
    m1, i1, m2, i2 = state['top']

    big = jnp.int32(1 << 30)
    ra = jnp.max(m1, axis=0, keepdims=True)
    ia = jnp.min(jnp.where(m1 == ra, i1, big), axis=0, keepdims=True)
    win = i1 == ia
    mm = jnp.where(win, m2, m1)
    ii = jnp.where(win, i2, i1)
    rb_ = jnp.max(mm, axis=0, keepdims=True)
    ib = jnp.min(jnp.where(mm == rb_, ii, big), axis=0, keepdims=True)
    sa = jnp.clip(ia[0, 0], 0, S - 1)
    sb = jnp.clip(ib[0, 0], 0, S - 1)

    def hrow(si, j):
        e, o = _unpk(jnp.broadcast_to(h_s[j, pl.ds(si // 2, 1), :], (8, 128)))
        return jnp.where(si % 2 == 0, e, o)

    xs = jnp.concatenate([jnp.concatenate([hrow(si, j) for j in range(NP)], axis=1) for si in (sa, sb)],
                         axis=0).astype(BF)

    hid = []
    for j in range(NF):
        g = _rbf(_dot(xs, _b16(wg32[j])))
        u = _rbf(_dot(xs, _b16(wu32[j])))
        g = _rbf(g * _rbf(jax.nn.sigmoid(g)))
        hid.append((g * u).astype(BF))
    hid = jnp.concatenate(hid, axis=1)
    rs = jnp.concatenate([jnp.broadcast_to(_rbf(jax.nn.sigmoid(ra)), (8, 1)),
                          jnp.broadcast_to(_rbf(jax.nn.sigmoid(rb_)), (8, 1))], axis=0)
    ys = [_rbf(_rbf(_dot(hid, _b16(wd32[j]))) * rs) for j in range(NP)]

    for c in out_cps:
        c.wait()

    def patch(si, slot):
        g0 = mo((si // 16) * 16, 16)
        ww = mo(g0 // 2, 8)
        rows = g0 + 2 * lax.broadcasted_iota(I32, (8, 128), 0)
        for j in range(NP):
            ya, yb = ys[j][0:8, :], ys[j][8:16, :]
            hp = _unpk(h_s[j, pl.ds(ww, 8), :])
            xp = _unpk(x32[j, pl.ds(ww, 8), :])
            res = []
            for par in range(2):
                upd = jnp.where(rows + par == sa, ya, jnp.where(rows + par == sb, yb, 0.0))
                res.append(xp[par] + mod_s[5 * NP + j] * _rbf(hp[par] + upd))
            pst32[slot * 8:slot * 8 + 8, j * 128:(j + 1) * 128] = _pk(res[0], res[1])
        return pltpu.make_async_copy(pst_s.at[pl.ds(slot * 16, 16), :], out_hbm.at[pl.ds(g0, 16), :], sem_s.at[slot])

    ca = patch(sa, 0)
    cb = patch(sb, 1)
    ca.start()

    @pl.when(sa // 16 != sb // 16)
    def _():
        cb.start()
        cb.wait()

    ca.wait()


@jax.jit
def pallas_adaLN_cond__mha_block_cached__moe_arch_mod__prompt_kernel(
    A_x: jax.Array,
    A_k_cache: jax.Array,
    A_v_cache: jax.Array,
    A_wq: jax.Array,
    A_wo: jax.Array,
    B_x: jax.Array,
    B_w_r: jax.Array,
    B_w_gate: jax.Array,
    B_w_up: jax.Array,
    B_w_down: jax.Array,
    c: jax.Array,
    w_mod: jax.Array,
):
    del B_x
    hbm = pl.BlockSpec(memory_space=pl.ANY)
    dma = pltpu.SemaphoreType.DMA
    rq = pltpu.VMEM((5, 256, 128), I32)
    lo = pltpu.VMEM((5 * 16, R // 2, 128), I32)
    out = pl.pallas_call(
        _kernel,
        out_shape=jax.ShapeDtypeStruct((S, D), BF),
        in_specs=[hbm] * 11,
        out_specs=hbm,
        scratch_shapes=[
            pltpu.VMEM((NP, S, 128), BF),
            pltpu.VMEM((NP, S, 128), BF),
            pltpu.VMEM((NSL * 7 * 4, R // 2, 128), I32),
            pltpu.VMEM((NP, S // 2, 128), I32),
            pltpu.VMEM((H, S // 2, 128), I32),
            pltpu.VMEM((H, D, 128), BF),
            pltpu.VMEM((NP, H * DH, 128), BF),
            pltpu.VMEM((5 * 4, 1024, 128), I32),
            pltpu.VMEM((NF, D, 128), BF),
            pltpu.VMEM((NF, D, 128), BF),
            pltpu.VMEM((NP, FF, 128), BF),
            pltpu.VMEM((6 * NP, D, 128), BF),
            pltpu.VMEM((2, HPI, S, DH), BF),
            pltpu.VMEM((2, HPI, S, DH), BF),
            pltpu.VMEM((6 * NP, 8, 128), F32),
            pltpu.VMEM((NP, 2 * R, 128), F32),
            pltpu.VMEM((NP, 2 * R, 128), F32),
            lo, lo, rq, rq, rq, rq, rq, rq,
            pltpu.VMEM((1, D), BF),
            pltpu.VMEM((D,), BF),
            pltpu.VMEM((D, 128), F32),
            pltpu.VMEM((2, D // 2, 128), F32),
            pltpu.VMEM((32, D), BF),
            dma((len(X_STAGES) - 1,)), dma((1 + H // 2,)), dma((1,)), dma((1,)), dma((5,)),
            dma((2,)), dma((2,)), dma((12,)), dma((2,)),
        ],
        compiler_params=pltpu.CompilerParams(vmem_limit_bytes=124 * 1024 * 1024),
    )(A_x.reshape(S, D), A_k_cache.reshape(H, S, DH), A_v_cache.reshape(H, S, DH), A_wq, A_wo,
      B_w_r, B_w_gate, B_w_up, B_w_down, c, w_mod)
    return out.reshape(1, S, D)
```

```python
import jax
import jax.numpy as jnp
import jax.experimental.pallas as pl
import jax.experimental.pallas.tpu as pltpu
from jax import lax

BF = jnp.bfloat16
F32 = jnp.float32
I32 = jnp.int32

S = 2048
D = 1024
H = 32
DH = 128
FF = 3584
NP = D // 128
NF = FF // 128
EPS = 1e-5
QSCALE = float(DH ** -0.5 * 1.4426950408889634)
L_LO = 2.0 ** -30
L_HI = 2.0 ** 40

XB = 256
NXB = S // XB
R = 64
NSL = S // (2 * R)
P0 = 4
PPI = 2
BQ = 256
HPI = 2
WQ_SPLIT = 2 * P0 + 2 + 4 * PPI
LO_SPAN, LO_FIRST, LN_SPAN, LN_ST = 24, 12, 16, 3
X_STAGES = (0, 128, 512, 1024, 2048)
DPI = 2

NN = (((1,), (0,)), ((), ()))
NT = (((1,), (1,)), ((), ()))


def _b16(x):
    return pltpu.bitcast(x, BF)


def _i32(x):
    return pltpu.bitcast(x, I32)


def _rbf(x):
    return x.astype(BF).astype(F32)


def _dot(a, b, dims=NN):
    return lax.dot_general(a, b, dims, preferred_element_type=F32)


def _unpk(w):
    return (pltpu.unpack_elementwise(w, index=0, packed_dtype=BF, unpacked_dtype=F32),
            pltpu.unpack_elementwise(w, index=1, packed_dtype=BF, unpacked_dtype=F32))


def _pk(even, odd):
    return pltpu.bitcast(pltpu.pack_elementwise([even, odd], packed_dtype=BF), I32)


def _zero_after(v):
    i = pltpu.bitcast(v[0:8, :], I32)
    return lax.shift_right_logical(lax.shift_right_logical(i, 31), 1)


def _tie(x, z):
    if z is None:
        return x
    return jnp.concatenate([x[r:r + 8] + z for r in range(0, x.shape[0], 8)], axis=0)


def _tief(x, z):
    return x if z is None else pltpu.bitcast(pltpu.bitcast(x, I32) + z[:, 0:1], F32)


def _ln_parts(parts, z1=None, z2=None):
    tot = parts[0]
    for p in parts[1:]:
        tot = tot + p
    m = _tief(jnp.sum(tot, axis=1, keepdims=True) * (1.0 / D), z1)
    dfs = [p - m for p in parts]
    sq = dfs[0] * dfs[0]
    for d in dfs[1:]:
        sq = sq + d * d
    v = _rbf(_rbf(jnp.sum(sq, axis=1, keepdims=True) * (1.0 / D)) + EPS)
    rs = lax.rsqrt(v)
    s = _rbf(v * rs)
    return dfs, _tief(rs * (2.0 - s * rs), z2)


def _strassen(prod):
    m1 = prod(0)
    m5 = prod(4)
    m4 = prod(3)
    m7 = prod(6)
    c11 = m1 + m4 - m5 + m7
    m3 = prod(2)
    c12 = m3 + m5
    m2 = prod(1)
    c21 = m2 + m4
    m6 = prod(5)
    c22 = m1 - m2 + m3 + m6
    return c11, c12, c21, c22


def _kernel(x_hbm, k_hbm, v_hbm, wq_hbm, wo_hbm, wr_hbm, wg_hbm, wu_hbm, wd_hbm, c_hbm, wm_hbm,
            out_hbm,
            x_s, x1_s, out_s, lq_s, h_s, q_s, wq_s, wo_s, ro_s, wg_s, wu_s, wd_s, wm_s, k_s, v_s, mod_s,
            t0_s, t1_s, lo0_s, lo1_s, ra_s, rb_s, rc_s, rd_s, re_s, rf_s, c_s, wr_s, ccol_s, cc2_s, pst_s,
            sem_x, sem_wq, sem_wo, sem_mlp, sem_m, sem_k, sem_v, sem_o, sem_s):
    wq32 = wq_s.bitcast(I32)
    wo32 = wo_s.bitcast(I32)
    wm32 = wm_s.bitcast(I32)
    k32 = k_s.bitcast(I32)
    v32 = v_s.bitcast(I32)
    x32 = x_s.bitcast(I32)
    x132 = x1_s.bitcast(I32)
    out32 = out_s.bitcast(I32)
    pst32 = pst_s.bitcast(I32)

    def mo(i, m):
        return i if isinstance(i, int) else pl.multiple_of(i, m)

    def col(j):
        return pl.ds(mo(j * 128, 128), 128)

    def cp_x(st, j):
        r0, n = X_STAGES[st], X_STAGES[st + 1] - X_STAGES[st]
        return pltpu.make_async_copy(x_hbm.at[pl.ds(r0, n), col(j)], x_s.at[j, pl.ds(r0, n), :], sem_x.at[st])

    def cp_wq(h, g):
        src = h if not isinstance(h, int) or h < H else h - 2
        return pltpu.make_async_copy(wq_hbm.at[:, col(src)], wq_s.at[h], sem_wq.at[g])

    def wq_group(h):
        if h < 2 * P0:
            return 0
        if h < 2 * P0 + 2:
            return 1
        return 2 + (h - 2 * P0 - 2) // (2 * PPI)

    def cp_m(j, g):
        return pltpu.make_async_copy(wm_hbm.at[:, col(j)], wm_s.at[j], sem_m.at[g])

    def m_panel(i):
        return i // 4 + 4 * (i % 4)

    def cp_wo(j):
        return pltpu.make_async_copy(wo_hbm.at[:, col(j)], wo_s.at[j], sem_wo.at[0])

    NG = H // HPI

    def cp_mlp(g):
        return [pltpu.make_async_copy(src.at[pl.ds(mo(g * n, 16), n), :], dst.at[pl.ds(mo(g * n, 16), n), :], sem_mlp.at[0])
                for src, dst, n in ((wg_hbm, wg_s, D // NG), (wu_hbm, wu_s, D // NG), (wd_hbm, wd_s, FF // NG))]

    def cp_kv(g, slot):
        return (pltpu.make_async_copy(k_hbm.at[pl.ds(mo(g * HPI, HPI), HPI)], k_s.at[slot], sem_k.at[slot]),
                pltpu.make_async_copy(v_hbm.at[pl.ds(mo(g * HPI, HPI), HPI)], v_s.at[slot], sem_v.at[slot]))

    def cp_o(r0, n, j, i):
        return pltpu.make_async_copy(out_s.at[j, pl.ds(r0, n), :], out_hbm.at[pl.ds(r0, n), col(j)], sem_o.at[i])

    cp_c = pltpu.make_async_copy(c_hbm, c_s, sem_s.at[0])
    cp_r = pltpu.make_async_copy(wr_hbm, wr_s, sem_s.at[1])
    cp_c.start()

    @pl.loop(0, NP)
    def _(j):
        cp_x(0, j).start()

    @pl.loop(0, 2 * P0)
    def _(h):
        cp_wq(h, 0).start()

    @pl.loop(0, 2 * NP)
    def _(i):
        cp_m(m_panel(i), i // 4).start()

    @pl.loop(0, NP)
    def _(j):
        cp_x(1, j).start()

    def rq_step(p, dst, r0, z=None):
        a, b = 2 * p, 2 * p + 1

        def ld(h, half):
            return _unpk(_tie(wq32[h, pl.ds(half * 256 + r0, 32), :], z))
        b11, b12, b21, b22 = ld(a, 0), ld(b, 0), ld(a, 1), ld(b, 1)
        for i, (u, v, sg) in enumerate(((b11, b22, 1), (b12, b22, -1), (b21, b11, -1), (b11, b12, 1), (b21, b22, 1))):
            dst[i, r0:r0 + 32, :] = _pk(u[0] + v[0], u[1] + v[1]) if sg > 0 else _pk(u[0] - v[0], u[1] - v[1])

    def rq_combos(p, dst):
        for r0 in range(0, 256, 32):
            rq_step(p, dst, r0)

    def lq_store(s, kc, hs, w0, nw):
        ops = [(a11 + a22, a21 + a22, a11, a22, a11 + a12, a21 - a11, a12 - a22) for a11, a12, a21, a22 in hs]
        for i in range(7):
            lq_s[(s * 7 + i) * 4 + kc, w0:w0 + nw, :] = _pk(ops[0][i], ops[1][i])

    def ln1(s, w0, nw, z, z1, z2):
        hs = [[], []]
        for half in range(2):
            ww = s * R + half * (R // 2) + w0
            xs = [_unpk(_tie(x32[j, ww:ww + nw, :], z)) for j in range(NP)]
            for par in range(2):
                ds, inv = _ln_parts([x_[par] for x_ in xs], z1, z2)
                hs[par].append([(ds[j] * inv) * mod_s[NP + j, 0:1, :] + mod_s[j, 0:1, :] for j in range(NP)])
        for kc in range(4):
            lq_store(s, kc, [(hs[par][0][kc], hs[par][0][kc + 4], hs[par][1][kc], hs[par][1][kc + 4])
                             for par in range(2)], w0, nw)

    def q_slab(p, rsrc, s):
        a, b = 2 * p, 2 * p + 1
        toks = []

        def prod(i):
            lhs = jnp.concatenate([_b16(lq_s[(s * 7 + i) * 4 + kc]) for kc in range(4)], axis=1)
            if i == 1:
                w = wq32[a, 0:256, :]
            elif i == 4:
                w = wq32[b, 256:512, :]
            else:
                w = rsrc[{0: 0, 2: 1, 3: 2, 5: 3, 6: 4}[i]]
            m = _dot(lhs, _b16(w))
            toks.append(m)
            return m

        c11, c12, c21, c22 = _strassen(prod)
        w0 = mo(s * R, R)
        q_s[a, pl.ds(w0, R // 2), :] = _i32(c11.astype(BF))
        q_s[b, pl.ds(w0, R // 2), :] = _i32(c12.astype(BF))
        q_s[a, pl.ds(w0 + R // 2, R // 2), :] = _i32(c21.astype(BF))
        q_s[b, pl.ds(w0 + R // 2, R // 2), :] = _i32(c22.astype(BF))
        return toks

    cp_c.wait()
    for j in range(NP):
        cp_x(0, j).wait()
    cf = c_s[...].astype(F32)
    sc = _rbf(cf * _rbf(jax.nn.sigmoid(cf)))
    sc16 = jnp.broadcast_to(sc, (16, D)).astype(BF)
    for half in range(2):
        xs = [_unpk(x32[j, half * 32:half * 32 + 32, :]) for j in range(NP)]
        for par in range(2):
            ds, inv = _ln_parts([x_[par] for x_ in xs])
            for j in range(NP):
                t0_s[j, par * 64 + half * 32:par * 64 + half * 32 + 32, :] = ds[j] * inv
    scb = jnp.broadcast_to(sc, (128, D))
    for j in range(NP):
        ccol_s[j * 128:(j + 1) * 128, :] = scb[:, j * 128:(j + 1) * 128].T
    ce_s, co_s = cc2_s.at[0], cc2_s.at[1]
    ce_s[...] = ccol_s[pl.ds(0, D // 2, stride=2), :]
    co_s[...] = ccol_s[pl.ds(1, D // 2, stride=2), :]

    for h in range(2 * P0):
        cp_wq(h, 0).wait()
    rsm = (ra_s, rb_s, rc_s, rd_s)
    for p in range(P0):
        rq_combos(p, rsm[p])

    for g in range(4):
        for i in range(4):
            cp_m(m_panel(4 * g + i), g).wait()
        hh = []
        for j in (g, g + 4):
            sa = _rbf(_dot(sc16, _b16(wm32[j]))[0:8, :]) * QSCALE
            ca = _rbf(1.0 + _rbf(_dot(sc16, _b16(wm32[NP + j]))[0:8, :])) * QSCALE
            mod_s[j] = sa
            mod_s[NP + j] = ca
            hh.append(t0_s[j] * ca[0:1, :] + sa[0:1, :])
        lq_store(0, g, [(hh[0][par * 64:par * 64 + 32], hh[1][par * 64:par * 64 + 32],
                         hh[0][par * 64 + 32:par * 64 + 64], hh[1][par * 64 + 32:par * 64 + 64])
                        for par in range(2)], 0, 32)

    NPAIR = H // 2
    NB = (NPAIR - P0) // PPI
    rpp = (re_s, rf_s)
    for s in range(NSL):
        nxt = s + 1
        if nxt < NSL and nxt * 2 * R in X_STAGES:
            st = X_STAGES.index(nxt * 2 * R)
            for j in range(NP):
                cp_x(st, j).wait()
        if s == NSL - 1:
            for h in range(2 * P0, 2 * P0 + 2):
                cp_wq(h, 1).wait()
        toks = []
        for p in range(P0):
            toks += q_slab(p, rsm[p], s)
            if p > 0:
                continue
            if s == 0:
                for j in range(NP):
                    cp_x(2, j).start()
            if s == 3:
                for j in range(NP):
                    cp_x(3, j).start()
            if s == 7:
                for h in range(2 * P0, WQ_SPLIT):
                    cp_wq(h, wq_group(h)).start()
            if s == NSL - 1:
                for h in range(WQ_SPLIT, H + 2):
                    cp_wq(h, wq_group(h)).start()
                cp_r.start()
        if nxt < NSL:
            npc = R // 16
            for i in range(npc):
                zs = [_zero_after(toks[int((0.105 * i + d) * len(toks))]) for d in (0.0, 0.12, 0.24)]
                ln1(nxt, i * 8, 8, *zs)
        else:
            for i in range(8):
                rq_step(P0, rpp[0], i * 32, _zero_after(toks[i * len(toks) // 10]))

    def phase_b(g, carry):
        p0 = P0 + PPI * g
        for h in range(2 * PPI):
            cp_wq(2 * p0 + 2 + h, 2 + g).wait()

        @pl.when(g == 0)
        def _():
            for c in cp_kv(0, 0):
                c.start()
            for j in range(NP):
                cp_wo(j).start()
            for j in range(2 * NP, 6 * NP):
                cp_m(j, 4).start()

        for u in range(PPI):
            cur, nxt = rpp[u % 2], rpp[(u + 1) % 2]
            p = p0 + u
            for s in range(NSL):
                toks = q_slab(p, cur, s)
                if 1 <= s <= 8:
                    rq_step(p + 1, nxt, (s - 1) * 32, _zero_after(toks[0]))
        return carry

    lax.fori_loop(0, NB, phase_b, 0)

    for j in range(NP):
        cp_wo(j).wait()

    for j in range(2 * NP, 6 * NP):
        cp_m(j, 4).wait()

    def ro_job(g, n, r0, z):
        w0 = mo(g * 64, 64)

        def ld(j, half):
            return _unpk(_tie(wo32[j, pl.ds(w0 + half * 1024 + r0, 16), :], z))
        b11, b12, b21, b22 = ld(n, 0), ld(n + 4, 0), ld(n, 1), ld(n + 4, 1)
        for i, (u, v, sg) in enumerate(((b11, b22, 1), (b12, b22, -1), (b21, b11, -1), (b11, b12, 1), (b21, b22, 1))):
            ro_s[i * 4 + n, pl.ds(w0 + r0, 16), :] = (_pk(u[0] + v[0], u[1] + v[1]) if sg > 0
                                                     else _pk(u[0] - v[0], u[1] - v[1]))

    mst = {}

    def mod_job(j, r, z):
        we, wo_ = _unpk(_tie(wm32[j, r:r + 64, :], z))
        t = we * ce_s[r:r + 64, :] + wo_ * co_s[r:r + 64, :]
        t = jnp.sum(t.reshape(8, 8, 128), axis=0)
        mst['acc'] = t if r == 0 else mst['acc'] + t
        if r == 448:
            v = _rbf(jnp.sum(mst['acc'], axis=0, keepdims=True))
            v = jnp.where(j // NP == 4, _rbf(1.0 + v), v)
            mod_s[j] = jnp.broadcast_to(v, (8, 128))

    def lo_combos(w0, r, dst, g, z):
        def ld(h, half):
            return _unpk(_tie(q_s[h, pl.ds(mo(w0 + half * (r // 2), r // 2), r // 2), :], z))
        a11, a12, a21, a22 = ld(g, 0), ld(g + 16, 0), ld(g, 1), ld(g + 16, 1)
        for i, (u, v, sg) in enumerate(((a11, a22, 1), (a21, a22, 1), (a11, a12, 1), (a21, a11, -1), (a12, a22, -1))):
            dst[i * 16 + g, 0:r // 2, :] = (_pk(u[0] + v[0], u[1] + v[1]) if sg > 0
                                            else _pk(u[0] - v[0], u[1] - v[1]))

    def attn_group(g, carry):
        lmin, lmax, osum = carry
        slot = g % 2
        for c in cp_kv(g, slot):
            c.wait()
        ja = [lambda z, n=n, r0=r0: ro_job(g, n, r0, z) for n in range(4) for r0 in range(0, 64, 16)]
        jb = [lambda z, jj=jj, r=r: mod_job(2 * NP + 2 * g + jj, r, z) for jj in range(2) for r in range(0, 512, 64)]
        jobs = [x for pair in zip(ja, jb) for x in pair]
        nch = HPI * (S // BQ)
        ntok = (nch - 1) * 4
        tc = 0
        for hh in range(HPI):
            h = g * HPI + hh
            k = _b16(k32[slot, hh])
            v = _b16(v32[slot, hh])
            for ci in range(S // BQ):
                q = _b16(q_s[h, pl.ds(ci * BQ // 2, BQ // 2), :])
                s = _dot(q, k, NT)
                if hh == 0 and ci == 0:
                    for c in cp_kv((g + 1) % NG, 1 - slot):
                        c.start()
                    for c in cp_mlp(g):
                        c.start()
                for tt in range(4):
                    z = _zero_after(s[0:8, tt * 512:tt * 512 + 128])
                    todo = jobs[tc * len(jobs) // ntok:(tc + 1) * len(jobs) // ntok]
                    for f in todo:
                        f(z)
                    tc += 1
                p = jnp.exp2(s)
                l = jnp.sum(p, axis=1, keepdims=True)
                r0_ = pl.reciprocal(l, approx=True)
                o = _dot(p.astype(BF), v) * (r0_ * (2.0 - l * r0_))
                q_s[h, pl.ds(ci * BQ // 2, BQ // 2), :] = _i32(o.astype(BF))
                for t in range(BQ // 8):
                    lt = l[t * 8:(t + 1) * 8]
                    lmin = jnp.minimum(lmin, lt)
                    lmax = jnp.maximum(lmax, lt)
                    osum = osum + o[t * 8:(t + 1) * 8]
        return lmin, lmax, osum

    init = (jnp.full((8, 1), 3e38, F32), jnp.zeros((8, 1), F32), jnp.zeros((8, 128), F32))
    lmin, lmax, osum = lax.fori_loop(0, NG, attn_group, init)

    def safe_attention():
        def safe_pair(p, carry):
            rq_combos(p, re_s)

            def qs(s, c2):
                q_slab(p, re_s, s)
                return c2

            lax.fori_loop(0, NSL, qs, 0)

            def one_head(hh, c2):
                h = 2 * p + hh
                ck = pltpu.make_async_copy(k_hbm.at[h], k_s.at[1, 0], sem_k.at[1])
                cv = pltpu.make_async_copy(v_hbm.at[h], v_s.at[1, 0], sem_v.at[1])
                ck.start()
                cv.start()
                ck.wait()
                cv.wait()

                def chunk(ci, c3):
                    w0 = mo(ci * 64, 64)
                    q = _b16(q_s[h, pl.ds(w0, 64), :])
                    s = _dot(q, _b16(k32[1, 0]), NT)
                    p_ = jnp.exp2(s - jnp.max(s, axis=1, keepdims=True))
                    l = jnp.sum(p_, axis=1, keepdims=True)
                    o = _dot(p_.astype(BF), _b16(v32[1, 0])) * (1.0 / l)
                    q_s[h, pl.ds(w0, 64), :] = _i32(o.astype(BF))
                    return c3

                lax.fori_loop(0, S // 128, chunk, 0)
                return c2

            lax.fori_loop(0, 2, one_head, 0)
            return carry

        lax.fori_loop(0, NPAIR, safe_pair, 0)

    lo = jnp.min(lmin)
    hi = jnp.max(lmax)
    fin = jnp.max(jnp.where(jnp.abs(osum) < 3e38, 0.0, 1.0))
    bad = jnp.logical_or(jnp.logical_or(jnp.logical_not(lo >= L_LO), jnp.logical_not(hi <= L_HI)), fin > 0.5)
    pl.when(bad)(safe_attention)

    cp_r.wait()
    wr = wr_s[...].astype(F32).reshape(1, D)
    cw = [mod_s[4 * NP + j, 0:1, :] * wr[:, j * 128:(j + 1) * 128] for j in range(NP)]
    sw = mod_s[3 * NP, 0:1, :] * wr[:, 0:128]
    for j in range(1, NP):
        sw = sw + mod_s[3 * NP + j, 0:1, :] * wr[:, j * 128:(j + 1) * 128]
    sw = jnp.sum(sw, axis=1, keepdims=True)

    def o_slab(w0, r, lsrc, t_ref, side, split=False, first=False):
        cnt = [0]
        prods = []
        for n in range(4):
            def prod(i, n=n):
                if i == 2:
                    pan = [q_s[g, pl.ds(mo(w0, r // 2), r // 2), :] for g in range(16)]
                elif i == 3:
                    pan = [q_s[g + 16, pl.ds(mo(w0 + r // 2, r // 2), r // 2), :] for g in range(16)]
                else:
                    li = {0: 0, 1: 1, 4: 2, 5: 3, 6: 4}[i]
                    pan = [lsrc[li * 16 + g, 0:r // 2, :] for g in range(16)]
                lhs = jnp.concatenate([_b16(a) for a in pan], axis=1)
                if i == 1:
                    w = wo32[n, 0:1024, :]
                elif i == 4:
                    w = wo32[n + 4, 1024:2048, :]
                else:
                    w = ro_s[{0: 0, 2: 1, 3: 2, 5: 3, 6: 4}[i] * 4 + n]
                m = _dot(lhs, _b16(w))
                side(cnt[0], m)
                cnt[0] += 1
                return m
            prods.append(prod)
        if first:
            for n in range(4):
                t_ref[n, r:2 * r, :] = prods[n](3)
                t_ref[n + 4, 0:r, :] = prods[n](2)
            for n in range(4):
                m1, m5, m2 = prods[n](0), prods[n](4), prods[n](1)
                m4, m3 = t_ref[n, r:2 * r, :], t_ref[n + 4, 0:r, :]
                t_ref[n, 0:r, :] = m1 + m4 - m5 + prods[n](6)
                t_ref[n + 4, 0:r, :] = m3 + m5
                t_ref[n, r:2 * r, :] = m2 + m4
                t_ref[n + 4, r:2 * r, :] = m1 - m2 + m3 + prods[n](5)
            return
        for n in range(4):
            prod = prods[n]
            if split:
                m1, m5, m4, m7, m3 = prod(0), prod(4), prod(3), prod(6), prod(2)
                c11, c12, c21, c22 = m1 + m4 - m5 + m7, m3 + m5, m4, m1 + m3
            else:
                c11, c12, c21, c22 = _strassen(prod)
            t_ref[n, 0:r, :] = c11
            t_ref[n + 4, 0:r, :] = c12
            t_ref[n, r:2 * r, :] = c21
            t_ref[n + 4, r:2 * r, :] = c22
        if split:
            for n in range(4):
                m2, m6 = prods[n](1), prods[n](5)
                t_ref[n, r:2 * r, :] = t_ref[n, r:2 * r, :] + m2
                t_ref[n + 4, r:2 * r, :] = t_ref[n + 4, r:2 * r, :] + (m6 - m2)

    state = {}

    def ln2(rr, t_ref, p0, z, z1=None, z2=None):
        m1, i1, m2, i2 = state['top']
        ww = mo(rr // 2, 8)
        x1 = [[], []]
        for j in range(NP):
            xe, xo = _unpk(_tie(x32[j, pl.ds(ww, 8), :], z))
            ga = mod_s[2 * NP + j]
            e = xe + t_ref[j, pl.ds(p0, 8, stride=2), :] * ga
            o = xo + t_ref[j, pl.ds(p0 + 1, 8, stride=2), :] * ga
            x132[j, pl.ds(ww, 8), :] = _pk(e, o)
            x1[0].append(e)
            x1[1].append(o)
        hs, os_ = [], []
        for par in range(2):
            ds, inv = _ln_parts(x1[par], z1, z2)
            rd = ds[0] * cw[0]
            for j in range(1, NP):
                rd = rd + ds[j] * cw[j]
            v = _rbf(jnp.sum(rd, axis=1, keepdims=True) * inv + sw)
            hj = [(ds[j] * inv) * mod_s[4 * NP + j] + mod_s[3 * NP + j] for j in range(NP)]
            hs.append(hj)
            os_.append([x1[par][j] + mod_s[5 * NP + j] * hj[j] for j in range(NP)])
            idx = 2 * sub + (rr + par)
            gt1 = v > m1
            gt2 = v > m2
            m2 = jnp.where(gt1, m1, jnp.where(gt2, v, m2))
            i2 = jnp.where(gt1, i1, jnp.where(gt2, idx, i2))
            m1 = jnp.where(gt1, v, m1)
            i1 = jnp.where(gt1, idx, i1)
        for j in range(NP):
            h_s[j, pl.ds(ww, 8), :] = _pk(hs[0][j], hs[1][j])
            out32[j, pl.ds(ww, 8), :] = _pk(os_[0][j], os_[1][j])
        state['top'] = (m1, i1, m2, i2)

    ninf = jnp.full((8, 1), -jnp.inf, F32)
    sub = lax.broadcasted_iota(I32, (8, 1), 0)
    tb = (t0_s, t1_s)
    lb = (lo0_s, lo1_s)

    def d_step(row, r, slot, r_next, r_prev, split=False, first=False):
        jobs = []
        if r_next:
            g0 = LO_FIRST if first else 0
            for g in range(16):
                jobs.append(((g0 + g * (LO_SPAN if not first else 27 - g0) // 16,),
                             lambda z, g=g: lo_combos((row + 2 * r) // 2, r_next, lb[1 - slot], g, z)))
        if r_prev:
            npc = 2 * r_prev // 16
            for i in range(npc):
                k = (LO_FIRST if first else 0) + i * (LN_SPAN // 2 if first else LN_SPAN) // npc
                jobs.append(((k, k + LN_ST, k + 2 * LN_ST),
                             lambda *z, i=i: ln2(row - 2 * r_prev + i * 16, tb[1 - slot], i * 16, *z)))
        if split:
            for i in range(r // 16):
                jobs.append(((20 + 2 * i, 21 + 2 * i, 22 + 2 * i),
                             lambda *z, i=i: ln2(row + i * 16, tb[slot], i * 16, *z)))
        zs = []

        def side(k, m):
            zs.append(_zero_after(m) if any(k in ks for ks, _ in jobs) else None)
            for ks, f in jobs:
                if ks[-1] == k:
                    f(*[zs[i] for i in ks])

        o_slab(row // 2, r, lb[slot], tb[slot], side, split, first)

    ND = (NSL - 2) // DPI
    OB = 4 * R
    last = (NSL - 1) * 2 * R

    def d_loop(i, top):
        state['top'] = top
        row = mo(2 * R + i * DPI * 2 * R, 2 * R)
        for u in range(DPI):
            d_step(row + u * 2 * R, R, (u + 1) % 2, R, R)
            if u % 2 == 1:
                for j in range(NP):
                    cp_o(mo(row + (u - 2) * 2 * R, OB), OB, j, 0).start()
        return state['top']

    state['top'] = (ninf, sub + S, ninf, sub + S + 8)
    for g in range(16):
        lo_combos(0, R, lb[0], g, None)
    d_step(0, R, 0, R, 0, first=True)
    if ND == 1:
        d_loop(0, state['top'])
    else:
        state['top'] = lax.fori_loop(0, ND, d_loop, state['top'])
    for g in range(16):
        lo_combos(last // 2, R // 2, lb[1], g, None)
    d_step(last, R // 2, 1, R // 2, R, first=True)
    d_step(last + R, R // 2, 0, 0, R // 2, split=True)
    for i in range(R // 32, R // 16):
        ln2(last + R + i * 16, tb[0], i * 16, None)
    out_cps = [cp_o(i * OB, OB, j, 0) for i in range((NSL - 2) // 2) for j in range(NP)]
    for j in range(NP):
        c = cp_o(last - 2 * R, 4 * R, j, 0)
        c.start()
        out_cps.append(c)
    m1, i1, m2, i2 = state['top']

    big = jnp.int32(1 << 30)
    ra = jnp.max(m1, axis=0, keepdims=True)
    ia = jnp.min(jnp.where(m1 == ra, i1, big), axis=0, keepdims=True)
    win = i1 == ia
    mm = jnp.where(win, m2, m1)
    ii = jnp.where(win, i2, i1)
    rb_ = jnp.max(mm, axis=0, keepdims=True)
    ib = jnp.min(jnp.where(mm == rb_, ii, big), axis=0, keepdims=True)
    sa = jnp.clip(ia[0, 0], 0, S - 1)
    sb = jnp.clip(ib[0, 0], 0, S - 1)

    def hrow(si, j):
        e, o = _unpk(jnp.broadcast_to(h_s[j, pl.ds(si // 2, 1), :], (8, 128)))
        return jnp.where(si % 2 == 0, e, o)

    xs = jnp.concatenate([jnp.concatenate([hrow(si, j) for j in range(NP)], axis=1) for si in (sa, sb)],
                         axis=0).astype(BF)

    for g in range(NG):
        for c in cp_mlp(g):
            c.wait()
    for c in cp_kv(0, NG % 2):
        c.wait()
    hid = []
    for j in range(NF):
        g = _rbf(_dot(xs, wg_s[:, j * 128:(j + 1) * 128]))
        u = _rbf(_dot(xs, wu_s[:, j * 128:(j + 1) * 128]))
        g = _rbf(g * _rbf(jax.nn.sigmoid(g)))
        hid.append((g * u).astype(BF))
    hid = jnp.concatenate(hid, axis=1)
    rs = jnp.concatenate([jnp.broadcast_to(_rbf(jax.nn.sigmoid(ra)), (8, 1)),
                          jnp.broadcast_to(_rbf(jax.nn.sigmoid(rb_)), (8, 1))], axis=0)
    ys = [_rbf(_rbf(_dot(hid, wd_s[:, j * 128:(j + 1) * 128])) * rs) for j in range(NP)]

    for c in out_cps:
        c.wait()

    def patch(si, slot):
        g0 = mo((si // 16) * 16, 16)
        ww = mo(g0 // 2, 8)
        rows = g0 + 2 * lax.broadcasted_iota(I32, (8, 128), 0)
        for j in range(NP):
            ya, yb = ys[j][0:8, :], ys[j][8:16, :]
            hp = _unpk(h_s[j, pl.ds(ww, 8), :])
            xp = _unpk(x132[j, pl.ds(ww, 8), :])
            res = []
            for par in range(2):
                upd = jnp.where(rows + par == sa, ya, jnp.where(rows + par == sb, yb, 0.0))
                res.append(xp[par] + mod_s[5 * NP + j] * _rbf(hp[par] + upd))
            pst32[slot * 8:slot * 8 + 8, j * 128:(j + 1) * 128] = _pk(res[0], res[1])
        return pltpu.make_async_copy(pst_s.at[pl.ds(slot * 16, 16), :], out_hbm.at[pl.ds(g0, 16), :], sem_s.at[slot])

    ca = patch(sa, 0)
    cb = patch(sb, 1)
    ca.start()

    @pl.when(sa // 16 != sb // 16)
    def _():
        cb.start()
        cb.wait()

    ca.wait()


@jax.jit
def pallas_adaLN_cond__mha_block_cached__moe_arch_mod__prompt_kernel(
    A_x: jax.Array,
    A_k_cache: jax.Array,
    A_v_cache: jax.Array,
    A_wq: jax.Array,
    A_wo: jax.Array,
    B_x: jax.Array,
    B_w_r: jax.Array,
    B_w_gate: jax.Array,
    B_w_up: jax.Array,
    B_w_down: jax.Array,
    c: jax.Array,
    w_mod: jax.Array,
):
    del B_x
    hbm = pl.BlockSpec(memory_space=pl.ANY)
    dma = pltpu.SemaphoreType.DMA
    rq = pltpu.VMEM((5, 256, 128), I32)
    lo = pltpu.VMEM((5 * 16, R // 2, 128), I32)
    out = pl.pallas_call(
        _kernel,
        out_shape=jax.ShapeDtypeStruct((S, D), BF),
        in_specs=[hbm] * 11,
        out_specs=hbm,
        scratch_shapes=[
            pltpu.VMEM((NP, S, 128), BF),
            pltpu.VMEM((NP, S, 128), BF),
            pltpu.VMEM((NP, S, 128), BF),
            pltpu.VMEM((NSL * 7 * 4, R // 2, 128), I32),
            pltpu.VMEM((NP, S // 2, 128), I32),
            pltpu.VMEM((H, S // 2, 128), I32),
            pltpu.VMEM((H + 2, D, 128), BF),
            pltpu.VMEM((NP, H * DH, 128), BF),
            pltpu.VMEM((5 * 4, 1024, 128), I32),
            pltpu.VMEM((D, FF), BF),
            pltpu.VMEM((D, FF), BF),
            pltpu.VMEM((FF, D), BF),
            pltpu.VMEM((6 * NP, D, 128), BF),
            pltpu.VMEM((2, HPI, S, DH), BF),
            pltpu.VMEM((2, HPI, S, DH), BF),
            pltpu.VMEM((6 * NP, 8, 128), F32),
            pltpu.VMEM((NP, 2 * R, 128), F32),
            pltpu.VMEM((NP, 2 * R, 128), F32),
            lo, lo, rq, rq, rq, rq, rq, rq,
            pltpu.VMEM((1, D), BF),
            pltpu.VMEM((D,), BF),
            pltpu.VMEM((D, 128), F32),
            pltpu.VMEM((2, D // 2, 128), F32),
            pltpu.VMEM((32, D), BF),
            dma((len(X_STAGES) - 1,)), dma((2 + (H // 2 - P0) // PPI,)), dma((1,)), dma((1,)), dma((5,)),
            dma((2,)), dma((2,)), dma((1,)), dma((2,)),
        ],
        compiler_params=pltpu.CompilerParams(vmem_limit_bytes=124 * 1024 * 1024),
    )(A_x.reshape(S, D), A_k_cache.reshape(H, S, DH), A_v_cache.reshape(H, S, DH), A_wq, A_wo,
      B_w_r, B_w_gate, B_w_up, B_w_down, c, w_mod)
    return out.reshape(1, S, D)
```

```python
import jax
import jax.numpy as jnp
import jax.experimental.pallas as pl
import jax.experimental.pallas.tpu as pltpu
from jax import lax

BF = jnp.bfloat16
F32 = jnp.float32
I32 = jnp.int32

S = 2048
D = 1024
H = 32
DH = 128
FF = 3584
NP = D // 128
NF = FF // 128
EPS = 1e-5
QSCALE = float(DH ** -0.5 * 1.4426950408889634)
L_LO = 2.0 ** -30
L_HI = 2.0 ** 40

XB = 256
NXB = S // XB
R = 64
NSL = S // (2 * R)
P0 = 8
IPI = 4
BQ = 256
HPI = 2
BLK = (0, 1, 2, 4, 6, 8)
LO_SPAN, LO_FIRST, LN_SPAN, LN_ST = 24, 12, 16, 3
X_STAGES = (0, 256, 512, 768, 1024, 2048)
DPI = 2

NN = (((1,), (0,)), ((), ()))
NT = (((1,), (1,)), ((), ()))


def _b16(x):
    return pltpu.bitcast(x, BF)


def _i32(x):
    return pltpu.bitcast(x, I32)


def _rbf(x):
    return x.astype(BF).astype(F32)


def _dot(a, b, dims=NN):
    return lax.dot_general(a, b, dims, preferred_element_type=F32)


def _unpk(w):
    return (pltpu.unpack_elementwise(w, index=0, packed_dtype=BF, unpacked_dtype=F32),
            pltpu.unpack_elementwise(w, index=1, packed_dtype=BF, unpacked_dtype=F32))


def _pk(even, odd):
    return pltpu.bitcast(pltpu.pack_elementwise([even, odd], packed_dtype=BF), I32)


def _zero_after(v):
    i = pltpu.bitcast(v[0:8, :], I32)
    return lax.shift_right_logical(lax.shift_right_logical(i, 31), 1)


def _tie(x, z):
    if z is None:
        return x
    return jnp.concatenate([x[r:r + 8] + z for r in range(0, x.shape[0], 8)], axis=0)


def _tief(x, z):
    return x if z is None else pltpu.bitcast(pltpu.bitcast(x, I32) + z[:, 0:1], F32)


def _ln_parts(parts, z1=None, z2=None):
    tot = parts[0]
    for p in parts[1:]:
        tot = tot + p
    m = _tief(jnp.sum(tot, axis=1, keepdims=True) * (1.0 / D), z1)
    dfs = [p - m for p in parts]
    sq = dfs[0] * dfs[0]
    for d in dfs[1:]:
        sq = sq + d * d
    v = _rbf(_rbf(jnp.sum(sq, axis=1, keepdims=True) * (1.0 / D)) + EPS)
    rs = lax.rsqrt(v)
    s = _rbf(v * rs)
    return dfs, _tief(rs * (2.0 - s * rs), z2)


def _strassen(prod):
    m1 = prod(0)
    m5 = prod(4)
    m4 = prod(3)
    m7 = prod(6)
    c11 = m1 + m4 - m5 + m7
    m3 = prod(2)
    c12 = m3 + m5
    m2 = prod(1)
    c21 = m2 + m4
    m6 = prod(5)
    c22 = m1 - m2 + m3 + m6
    return c11, c12, c21, c22


def _kernel(x_hbm, k_hbm, v_hbm, wq_hbm, wo_hbm, wr_hbm, wg_hbm, wu_hbm, wd_hbm, c_hbm, wm_hbm,
            out_hbm,
            x_s, x1_s, out_s, lq_s, h_s, q_s, wq_s, wo_s, ro_s, wg_s, wu_s, wd_s, wm_s, k_s, v_s, mod_s,
            t0_s, t1_s, lo0_s, lo1_s, re_s, rf_s, c_s, wr_s, ccol_s, cc2_s, cs2_s, b_s, pst_s,
            sem_x, sem_wq, sem_wo, sem_mlp, sem_m, sem_k, sem_v, sem_o, sem_s):
    wq32 = wq_s.bitcast(I32)
    wo32 = wo_s.bitcast(I32)
    wm32 = wm_s.bitcast(I32)
    k32 = k_s.bitcast(I32)
    v32 = v_s.bitcast(I32)
    x32 = x_s.bitcast(I32)
    x132 = x1_s.bitcast(I32)
    out32 = out_s.bitcast(I32)
    pst32 = pst_s.bitcast(I32)

    def mo(i, m):
        return i if isinstance(i, int) else pl.multiple_of(i, m)

    def col(j):
        return pl.ds(mo(j * 128, 128), 128)

    def cp_x(st, j):
        r0, n = X_STAGES[st], X_STAGES[st + 1] - X_STAGES[st]
        return pltpu.make_async_copy(x_hbm.at[pl.ds(r0, n), col(j)], x_s.at[j, pl.ds(r0, n), :], sem_x.at[st])

    def cp_wq(h, g):
        src = h if not isinstance(h, int) or h < H else h - 2
        return pltpu.make_async_copy(wq_hbm.at[:, col(src)], wq_s.at[h], sem_wq.at[g])

    def item(i):
        if isinstance(i, int):
            return (i, NSL // 2) if i < P0 else (P0 + (i - P0) // 2, (i - P0) % 2 * (NSL // 2))
        j = jnp.maximum(i - P0, 0)
        return (jnp.where(i < P0, i, P0 + j // 2), jnp.where(i < P0, NSL // 2, j % 2 * (NSL // 2)))

    NPAIR = H // 2
    NB = (P0 + 2 * (NPAIR - P0)) // IPI
    G_LOOP = P0 // IPI
    WQ_EXTRA = 2 + IPI * (NB - G_LOOP)

    NBLK = len(BLK) - 1

    def wq_group(h):
        p = h // 2
        if p < P0:
            return 0 if p == 0 else min(k for k in range(1, NBLK) if p <= BLK[k + 1])
        return NBLK if p == P0 else NBLK + 1 + (p - P0 - 1) // (IPI // 2)

    def cp_m(j, g):
        return pltpu.make_async_copy(wm_hbm.at[:, col(j)], wm_s.at[j], sem_m.at[g])

    def m_panel(i):
        return NP + i // 2 + 4 * (i % 2)

    def cp_wo(j):
        return pltpu.make_async_copy(wo_hbm.at[:, col(j)], wo_s.at[j], sem_wo.at[0])

    NG = H // HPI

    def cp_mlp(g):
        return [pltpu.make_async_copy(src.at[pl.ds(mo(g * n, 16), n), :], dst.at[pl.ds(mo(g * n, 16), n), :], sem_mlp.at[0])
                for src, dst, n in ((wg_hbm, wg_s, D // NG), (wu_hbm, wu_s, D // NG), (wd_hbm, wd_s, FF // NG))]

    def cp_kv(g, slot):
        return (pltpu.make_async_copy(k_hbm.at[pl.ds(mo(g * HPI, HPI), HPI)], k_s.at[slot], sem_k.at[slot]),
                pltpu.make_async_copy(v_hbm.at[pl.ds(mo(g * HPI, HPI), HPI)], v_s.at[slot], sem_v.at[slot]))

    def cp_o(r0, n, j, i):
        return pltpu.make_async_copy(out_s.at[j, pl.ds(r0, n), :], out_hbm.at[pl.ds(r0, n), col(j)], sem_o.at[i])

    cp_c = pltpu.make_async_copy(c_hbm, c_s, sem_s.at[0])
    cp_r = pltpu.make_async_copy(wr_hbm, wr_s, sem_s.at[1])
    cp_c.start()

    @pl.loop(0, 2)
    def _(h):
        cp_wq(h, 0).start()

    @pl.loop(0, NP)
    def _(i):
        cp_m(m_panel(i), i // 2).start()

    for st in range(4):
        @pl.loop(0, NP)
        def _(j):
            cp_x(st, j).start()

    for k in (1, 2):
        hs = [h for h in range(H + 2) if wq_group(h) == k]

        @pl.loop(hs[0], hs[-1] + 1)
        def _(h):
            cp_wq(h, k).start()

    @pl.loop(0, NP)
    def _(j):
        cp_x(4, j).start()

    bst = {}

    def rq_step(p, dst, r0, z=None, bias=False):
        a, b = 2 * p, 2 * p + 1

        def ld(h, half):
            return _unpk(_tie(wq32[h, pl.ds(half * 256 + r0, 32), :], z))
        b11, b12, b21, b22 = ld(a, 0), ld(b, 0), ld(a, 1), ld(b, 1)
        for i, (u, v, sg) in enumerate(((b11, b22, 1), (b12, b22, -1), (b21, b11, -1), (b11, b12, 1), (b21, b22, 1))):
            dst[i, r0:r0 + 32, :] = _pk(u[0] + v[0], u[1] + v[1]) if sg > 0 else _pk(u[0] - v[0], u[1] - v[1])
        if bias:
            sh = [cs2_s[par, half * 256 + r0:half * 256 + r0 + 32, :] for half in range(2) for par in range(2)]
            for h, up, dn in ((a, b11, b21), (b, b12, b22)):
                t = up[0] * sh[0] + up[1] * sh[1] + dn[0] * sh[2] + dn[1] * sh[3]
                t = (t[0:8] + t[8:16]) + (t[16:24] + t[24:32])
                bst[h is a] = t if r0 == 0 else bst[h is a] + t
                if r0 == 224:
                    b_s[h] = jnp.broadcast_to(jnp.sum(bst[h is a], axis=0, keepdims=True), (8, 128))

    def rq_combos(p, dst):
        for r0 in range(0, 256, 32):
            rq_step(p, dst, r0)

    def load_q(h, w0, nw):
        e, o = _unpk(q_s[h, pl.ds(w0, nw), :])
        b = jnp.concatenate([b_s[h]] * (nw // 8), axis=0)
        return _b16(_pk(e + b, o + b))

    def lq_store(s, kc, hs, w0, nw):
        ops = [(a11 + a22, a21 + a22, a11, a22, a11 + a12, a21 - a11, a12 - a22) for a11, a12, a21, a22 in hs]
        for i in range(7):
            lq_s[(s * 7 + i) * 4 + kc, w0:w0 + nw, :] = _pk(ops[0][i], ops[1][i])

    def ln1(s, w0, nw, z, z1, z2):
        hs = [[], []]
        for half in range(2):
            ww = s * R + half * (R // 2) + w0
            xs = [_unpk(_tie(x32[j, ww:ww + nw, :], z)) for j in range(NP)]
            for par in range(2):
                ds, inv = _ln_parts([x_[par] for x_ in xs], z1, z2)
                hs[par].append([(ds[j] * inv) * mod_s[NP + j, 0:1, :] for j in range(NP)])
        for kc in range(4):
            lq_store(s, kc, [(hs[par][0][kc], hs[par][0][kc + 4], hs[par][1][kc], hs[par][1][kc + 4])
                             for par in range(2)], w0, nw)

    def q_slab(p, rsrc, s):
        a, b = 2 * p, 2 * p + 1
        toks = []

        def prod(i):
            lhs = jnp.concatenate([_b16(lq_s[(s * 7 + i) * 4 + kc]) for kc in range(4)], axis=1)
            if i == 1:
                w = wq32[a, 0:256, :]
            elif i == 4:
                w = wq32[b, 256:512, :]
            else:
                w = rsrc[{0: 0, 2: 1, 3: 2, 5: 3, 6: 4}[i]]
            m = _dot(lhs, _b16(w))
            toks.append(m)
            return m

        c11, c12, c21, c22 = _strassen(prod)
        w0 = mo(s * R, R)
        q_s[a, pl.ds(w0, R // 2), :] = _i32(c11.astype(BF))
        q_s[b, pl.ds(w0, R // 2), :] = _i32(c12.astype(BF))
        q_s[a, pl.ds(w0 + R // 2, R // 2), :] = _i32(c21.astype(BF))
        q_s[b, pl.ds(w0 + R // 2, R // 2), :] = _i32(c22.astype(BF))
        return toks

    cp_c.wait()
    cf = c_s[...].astype(F32)
    sc = _rbf(cf * _rbf(jax.nn.sigmoid(cf)))
    sc16 = jnp.broadcast_to(sc, (16, D)).astype(BF)
    scb = jnp.broadcast_to(sc, (128, D))
    for j in range(NP):
        ccol_s[j * 128:(j + 1) * 128, :] = scb[:, j * 128:(j + 1) * 128].T
    ce_s, co_s = cc2_s.at[0], cc2_s.at[1]
    ce_s[...] = ccol_s[pl.ds(0, D // 2, stride=2), :]
    co_s[...] = ccol_s[pl.ds(1, D // 2, stride=2), :]

    for h in range(2):
        cp_wq(h, 0).wait()
    rp = (re_s, rf_s)
    rq_combos(0, rp[0])

    for g in range(4):
        for i in range(2):
            cp_m(m_panel(2 * g + i), g).wait()
        for j in (g, g + 4):
            mod_s[NP + j] = _rbf(1.0 + _rbf(_dot(sc16, _b16(wm32[NP + j]))[0:8, :])) * QSCALE

    npc = R // 16

    def ln1_spread(slabs, toks):
        n = len(slabs) * npc
        for i in range(n):
            zs = [_zero_after(toks[int((i + d) * (len(toks) - 1) / (n + 2))]) if toks else None for d in (0.0, 1.0, 2.0)]
            ln1(slabs[i // npc], i % npc * 8, 8, *zs)

    for st in range(4):
        for j in range(NP):
            cp_x(st, j).wait()
        toks = []
        for s in range(max(2 * st - 2, 0), 2 * st):
            toks += q_slab(0, rp[0], s)
        ln1_spread((2 * st, 2 * st + 1), [])
    for k in range(1, NBLK):
        toks = []
        for h in range(2 * NPAIR):
            if wq_group(h) == k:
                cp_wq(h, k).wait()
        if k == NBLK - 2:
            for j in range(NP):
                cp_x(4, j).wait()
        if k == NBLK - 1:
            for j in range(NP):
                cp_m(j, 4).wait()
            for j in range(NP):
                sa = _rbf(_dot(sc16, _b16(wm32[j]))[0:1, :]) * QSCALE
                ccol_s[j * 128:(j + 1) * 128, :] = jnp.broadcast_to(sa, (128, 128)).T
            for par in range(2):
                cs2_s[par] = ccol_s[pl.ds(par, D // 2, stride=2), :]
        if k == 1:
            for s in (6, 7):
                q_slab(0, rp[0], s)
            rq_combos(1, rp[1])
        for p in range(BLK[k], BLK[k + 1]):
            for s in range(NSL // 2):
                tk = q_slab(p, rp[p % 2], s)
                toks += tk
                rq_step(p + 1 if p + 1 < P0 else item(0)[0], rp[(p + 1) % 2], s * 32, _zero_after(tk[0]),
                        bias=p + 1 == P0)
            if p == BLK[k]:
                if k == 2:
                    for j in range(NP):
                        cp_m(j, 4).start()
                for h in range(6, H + 2):
                    if (None, 3 <= wq_group(h) < NBLK, wq_group(h) == NBLK, wq_group(h) > NBLK, False)[k]:
                        cp_wq(h, wq_group(h)).start()
        if k >= NBLK - 2:
            s0 = NSL // 4 * (k - NBLK + 4)
            ln1_spread(tuple(range(s0, s0 + NSL // 4)), toks)

    for h in (2 * P0, 2 * P0 + 1):
        cp_wq(h, NBLK).wait()
    cp_r.start()

    def phase_b(g, carry):
        @pl.when(g >= G_LOOP)
        def _():
            for h in range(IPI):
                cp_wq(2 * P0 + 2 + (g - G_LOOP) * IPI + h, NBLK + 1 + g - G_LOOP).wait()

        @pl.when(g == 0)
        def _():
            for c in cp_kv(0, 0):
                c.start()
            for j in range(NP):
                cp_wo(j).start()
            for j in range(2 * NP, 6 * NP):
                cp_m(j, 4).start()

        for u in range(IPI):
            p, s0 = item(g * IPI + u)
            pn, _ = item(g * IPI + u + 1)
            for s in range(NSL // 2):
                toks = q_slab(p, rp[(P0 + u) % 2], s0 + s)
                rq_step(pn, rp[(P0 + u + 1) % 2], s * 32, _zero_after(toks[0]), bias=True)
        return carry

    lax.fori_loop(0, NB, phase_b, 0)

    for j in range(NP):
        cp_wo(j).wait()

    for j in range(2 * NP, 6 * NP):
        cp_m(j, 4).wait()

    def ro_job(g, n, r0, z):
        w0 = mo(g * 64, 64)

        def ld(j, half):
            return _unpk(_tie(wo32[j, pl.ds(w0 + half * 1024 + r0, 16), :], z))
        b11, b12, b21, b22 = ld(n, 0), ld(n + 4, 0), ld(n, 1), ld(n + 4, 1)
        for i, (u, v, sg) in enumerate(((b11, b22, 1), (b12, b22, -1), (b21, b11, -1), (b11, b12, 1), (b21, b22, 1))):
            ro_s[i * 4 + n, pl.ds(w0 + r0, 16), :] = (_pk(u[0] + v[0], u[1] + v[1]) if sg > 0
                                                     else _pk(u[0] - v[0], u[1] - v[1]))

    mst = {}

    def mod_job(j, r, z):
        we, wo_ = _unpk(_tie(wm32[j, r:r + 64, :], z))
        t = we * ce_s[r:r + 64, :] + wo_ * co_s[r:r + 64, :]
        t = jnp.sum(t.reshape(8, 8, 128), axis=0)
        mst['acc'] = t if r == 0 else mst['acc'] + t
        if r == 448:
            v = _rbf(jnp.sum(mst['acc'], axis=0, keepdims=True))
            v = jnp.where(j // NP == 4, _rbf(1.0 + v), v)
            mod_s[j] = jnp.broadcast_to(v, (8, 128))

    def lo_combos(w0, r, dst, g, z):
        def ld(h, half):
            return _unpk(_tie(q_s[h, pl.ds(mo(w0 + half * (r // 2), r // 2), r // 2), :], z))
        a11, a12, a21, a22 = ld(g, 0), ld(g + 16, 0), ld(g, 1), ld(g + 16, 1)
        for i, (u, v, sg) in enumerate(((a11, a22, 1), (a21, a22, 1), (a11, a12, 1), (a21, a11, -1), (a12, a22, -1))):
            dst[i * 16 + g, 0:r // 2, :] = (_pk(u[0] + v[0], u[1] + v[1]) if sg > 0
                                            else _pk(u[0] - v[0], u[1] - v[1]))

    def attn_group(g, carry):
        lmin, lmax, osum = carry
        slot = g % 2
        for c in cp_kv(g, slot):
            c.wait()
        ja = [lambda z, n=n, r0=r0: ro_job(g, n, r0, z) for n in range(4) for r0 in range(0, 64, 16)]
        jb = [lambda z, jj=jj, r=r: mod_job(2 * NP + 2 * g + jj, r, z) for jj in range(2) for r in range(0, 512, 64)]
        jobs = [x for pair in zip(ja, jb) for x in pair]
        nch = HPI * (S // BQ)
        ntok = (nch - 1) * 4
        tc = 0
        for hh in range(HPI):
            h = g * HPI + hh
            k = _b16(k32[slot, hh])
            v = _b16(v32[slot, hh])
            for ci in range(S // BQ):
                q = load_q(h, ci * BQ // 2, BQ // 2)
                s = _dot(q, k, NT)
                if hh == 0 and ci == 0:
                    for c in cp_kv((g + 1) % NG, 1 - slot):
                        c.start()
                    for c in cp_mlp(g):
                        c.start()
                for tt in range(4):
                    z = _zero_after(s[0:8, tt * 512:tt * 512 + 128])
                    todo = jobs[tc * len(jobs) // ntok:(tc + 1) * len(jobs) // ntok]
                    for f in todo:
                        f(z)
                    tc += 1
                p = jnp.exp2(s)
                l = jnp.sum(p, axis=1, keepdims=True)
                r0_ = pl.reciprocal(l, approx=True)
                o = _dot(p.astype(BF), v) * (r0_ * (2.0 - l * r0_))
                q_s[h, pl.ds(ci * BQ // 2, BQ // 2), :] = _i32(o.astype(BF))
                for t in range(BQ // 8):
                    lt = l[t * 8:(t + 1) * 8]
                    lmin = jnp.minimum(lmin, lt)
                    lmax = jnp.maximum(lmax, lt)
                    osum = osum + o[t * 8:(t + 1) * 8]
        return lmin, lmax, osum

    init = (jnp.full((8, 1), 3e38, F32), jnp.zeros((8, 1), F32), jnp.zeros((8, 128), F32))
    lmin, lmax, osum = lax.fori_loop(0, NG, attn_group, init)

    def safe_attention():
        def safe_pair(p, carry):
            rq_combos(p, re_s)

            def qs(s, c2):
                q_slab(p, re_s, s)
                return c2

            lax.fori_loop(0, NSL, qs, 0)

            def one_head(hh, c2):
                h = 2 * p + hh
                ck = pltpu.make_async_copy(k_hbm.at[h], k_s.at[1, 0], sem_k.at[1])
                cv = pltpu.make_async_copy(v_hbm.at[h], v_s.at[1, 0], sem_v.at[1])
                ck.start()
                cv.start()
                ck.wait()
                cv.wait()

                def chunk(ci, c3):
                    w0 = mo(ci * 64, 64)
                    q = load_q(h, w0, 64)
                    s = _dot(q, _b16(k32[1, 0]), NT)
                    p_ = jnp.exp2(s - jnp.max(s, axis=1, keepdims=True))
                    l = jnp.sum(p_, axis=1, keepdims=True)
                    o = _dot(p_.astype(BF), _b16(v32[1, 0])) * (1.0 / l)
                    q_s[h, pl.ds(w0, 64), :] = _i32(o.astype(BF))
                    return c3

                lax.fori_loop(0, S // 128, chunk, 0)
                return c2

            lax.fori_loop(0, 2, one_head, 0)
            return carry

        lax.fori_loop(0, NPAIR, safe_pair, 0)

    lo = jnp.min(lmin)
    hi = jnp.max(lmax)
    fin = jnp.max(jnp.where(jnp.abs(osum) < 3e38, 0.0, 1.0))
    bad = jnp.logical_or(jnp.logical_or(jnp.logical_not(lo >= L_LO), jnp.logical_not(hi <= L_HI)), fin > 0.5)
    pl.when(bad)(safe_attention)

    cp_r.wait()
    wr = wr_s[...].astype(F32).reshape(1, D)
    cw = [mod_s[4 * NP + j, 0:1, :] * wr[:, j * 128:(j + 1) * 128] for j in range(NP)]
    sw = mod_s[3 * NP, 0:1, :] * wr[:, 0:128]
    for j in range(1, NP):
        sw = sw + mod_s[3 * NP + j, 0:1, :] * wr[:, j * 128:(j + 1) * 128]
    sw = jnp.sum(sw, axis=1, keepdims=True)

    def o_slab(w0, r, lsrc, t_ref, side, split=False, first=False):
        cnt = [0]
        prods = []
        for n in range(4):
            def prod(i, n=n):
                if i == 2:
                    pan = [q_s[g, pl.ds(mo(w0, r // 2), r // 2), :] for g in range(16)]
                elif i == 3:
                    pan = [q_s[g + 16, pl.ds(mo(w0 + r // 2, r // 2), r // 2), :] for g in range(16)]
                else:
                    li = {0: 0, 1: 1, 4: 2, 5: 3, 6: 4}[i]
                    pan = [lsrc[li * 16 + g, 0:r // 2, :] for g in range(16)]
                lhs = jnp.concatenate([_b16(a) for a in pan], axis=1)
                if i == 1:
                    w = wo32[n, 0:1024, :]
                elif i == 4:
                    w = wo32[n + 4, 1024:2048, :]
                else:
                    w = ro_s[{0: 0, 2: 1, 3: 2, 5: 3, 6: 4}[i] * 4 + n]
                m = _dot(lhs, _b16(w))
                side(cnt[0], m)
                cnt[0] += 1
                return m
            prods.append(prod)
        if first:
            for n in range(4):
                t_ref[n, r:2 * r, :] = prods[n](3)
                t_ref[n + 4, 0:r, :] = prods[n](2)
            for n in range(4):
                m1, m5, m2 = prods[n](0), prods[n](4), prods[n](1)
                m4, m3 = t_ref[n, r:2 * r, :], t_ref[n + 4, 0:r, :]
                t_ref[n, 0:r, :] = m1 + m4 - m5 + prods[n](6)
                t_ref[n + 4, 0:r, :] = m3 + m5
                t_ref[n, r:2 * r, :] = m2 + m4
                t_ref[n + 4, r:2 * r, :] = m1 - m2 + m3 + prods[n](5)
            return
        for n in range(4):
            prod = prods[n]
            if split:
                m1, m5, m4, m7, m3 = prod(0), prod(4), prod(3), prod(6), prod(2)
                c11, c12, c21, c22 = m1 + m4 - m5 + m7, m3 + m5, m4, m1 + m3
            else:
                c11, c12, c21, c22 = _strassen(prod)
            t_ref[n, 0:r, :] = c11
            t_ref[n + 4, 0:r, :] = c12
            t_ref[n, r:2 * r, :] = c21
            t_ref[n + 4, r:2 * r, :] = c22
        if split:
            for n in range(4):
                m2, m6 = prods[n](1), prods[n](5)
                t_ref[n, r:2 * r, :] = t_ref[n, r:2 * r, :] + m2
                t_ref[n + 4, r:2 * r, :] = t_ref[n + 4, r:2 * r, :] + (m6 - m2)

    state = {}

    def ln2(rr, t_ref, p0, z, z1=None, z2=None):
        m1, i1, m2, i2 = state['top']
        ww = mo(rr // 2, 8)
        x1 = [[], []]
        for j in range(NP):
            xe, xo = _unpk(_tie(x32[j, pl.ds(ww, 8), :], z))
            ga = mod_s[2 * NP + j]
            e = xe + t_ref[j, pl.ds(p0, 8, stride=2), :] * ga
            o = xo + t_ref[j, pl.ds(p0 + 1, 8, stride=2), :] * ga
            x132[j, pl.ds(ww, 8), :] = _pk(e, o)
            x1[0].append(e)
            x1[1].append(o)
        hs, os_ = [], []
        for par in range(2):
            ds, inv = _ln_parts(x1[par], z1, z2)
            rd = ds[0] * cw[0]
            for j in range(1, NP):
                rd = rd + ds[j] * cw[j]
            v = _rbf(jnp.sum(rd, axis=1, keepdims=True) * inv + sw)
            hj = [(ds[j] * inv) * mod_s[4 * NP + j] + mod_s[3 * NP + j] for j in range(NP)]
            hs.append(hj)
            os_.append([x1[par][j] + mod_s[5 * NP + j] * hj[j] for j in range(NP)])
            idx = 2 * sub + (rr + par)
            gt1 = v > m1
            gt2 = v > m2
            m2 = jnp.where(gt1, m1, jnp.where(gt2, v, m2))
            i2 = jnp.where(gt1, i1, jnp.where(gt2, idx, i2))
            m1 = jnp.where(gt1, v, m1)
            i1 = jnp.where(gt1, idx, i1)
        for j in range(NP):
            h_s[j, pl.ds(ww, 8), :] = _pk(hs[0][j], hs[1][j])
            out32[j, pl.ds(ww, 8), :] = _pk(os_[0][j], os_[1][j])
        state['top'] = (m1, i1, m2, i2)

    ninf = jnp.full((8, 1), -jnp.inf, F32)
    sub = lax.broadcasted_iota(I32, (8, 1), 0)
    tb = (t0_s, t1_s)
    lb = (lo0_s, lo1_s)

    def d_step(row, r, slot, r_next, r_prev, split=False, first=False):
        jobs = []
        if r_next:
            g0 = LO_FIRST if first else 0
            for g in range(16):
                jobs.append(((g0 + g * (LO_SPAN if not first else 27 - g0) // 16,),
                             lambda z, g=g: lo_combos((row + 2 * r) // 2, r_next, lb[1 - slot], g, z)))
        if r_prev:
            npc = 2 * r_prev // 16
            for i in range(npc):
                k = (LO_FIRST if first else 0) + i * (LN_SPAN // 2 if first else LN_SPAN) // npc
                jobs.append(((k, k + LN_ST, k + 2 * LN_ST),
                             lambda *z, i=i: ln2(row - 2 * r_prev + i * 16, tb[1 - slot], i * 16, *z)))
        if split:
            for i in range(r // 16):
                jobs.append(((20 + 2 * i, 21 + 2 * i, 22 + 2 * i),
                             lambda *z, i=i: ln2(row + i * 16, tb[slot], i * 16, *z)))
        zs = []

        def side(k, m):
            zs.append(_zero_after(m) if any(k in ks for ks, _ in jobs) else None)
            for ks, f in jobs:
                if ks[-1] == k:
                    f(*[zs[i] for i in ks])

        o_slab(row // 2, r, lb[slot], tb[slot], side, split, first)

    ND = (NSL - 2) // DPI
    OB = 4 * R
    last = (NSL - 1) * 2 * R

    def d_loop(i, top):
        state['top'] = top
        row = mo(2 * R + i * DPI * 2 * R, 2 * R)
        for u in range(DPI):
            d_step(row + u * 2 * R, R, (u + 1) % 2, R, R)
            if u % 2 == 1:
                for j in range(NP):
                    cp_o(mo(row + (u - 2) * 2 * R, OB), OB, j, 0).start()
        return state['top']

    state['top'] = (ninf, sub + S, ninf, sub + S + 8)
    for g in range(16):
        lo_combos(0, R, lb[0], g, None)
    d_step(0, R, 0, R, 0, first=True)
    if ND == 1:
        d_loop(0, state['top'])
    else:
        state['top'] = lax.fori_loop(0, ND, d_loop, state['top'])
    for g in range(16):
        lo_combos(last // 2, R // 2, lb[1], g, None)
    d_step(last, R // 2, 1, R // 2, R, first=True)
    d_step(last + R, R // 2, 0, 0, R // 2, split=True)
    for i in range(R // 32, R // 16):
        ln2(last + R + i * 16, tb[0], i * 16, None)
    out_cps = [cp_o(i * OB, OB, j, 0) for i in range((NSL - 2) // 2) for j in range(NP)]
    for j in range(NP):
        c = cp_o(last - 2 * R, 4 * R, j, 0)
        c.start()
        out_cps.append(c)
    m1, i1, m2, i2 = state['top']

    big = jnp.int32(1 << 30)
    ra = jnp.max(m1, axis=0, keepdims=True)
    ia = jnp.min(jnp.where(m1 == ra, i1, big), axis=0, keepdims=True)
    win = i1 == ia
    mm = jnp.where(win, m2, m1)
    ii = jnp.where(win, i2, i1)
    rb_ = jnp.max(mm, axis=0, keepdims=True)
    ib = jnp.min(jnp.where(mm == rb_, ii, big), axis=0, keepdims=True)
    sa = jnp.clip(ia[0, 0], 0, S - 1)
    sb = jnp.clip(ib[0, 0], 0, S - 1)

    def hrow(si, j):
        e, o = _unpk(jnp.broadcast_to(h_s[j, pl.ds(si // 2, 1), :], (8, 128)))
        return jnp.where(si % 2 == 0, e, o)

    xs = jnp.concatenate([jnp.concatenate([hrow(si, j) for j in range(NP)], axis=1) for si in (sa, sb)],
                         axis=0).astype(BF)

    for g in range(NG):
        for c in cp_mlp(g):
            c.wait()
    for c in cp_kv(0, NG % 2):
        c.wait()
    hid = []
    for j in range(NF):
        g = _rbf(_dot(xs, wg_s[:, j * 128:(j + 1) * 128]))
        u = _rbf(_dot(xs, wu_s[:, j * 128:(j + 1) * 128]))
        g = _rbf(g * _rbf(jax.nn.sigmoid(g)))
        hid.append((g * u).astype(BF))
    hid = jnp.concatenate(hid, axis=1)
    rs = jnp.concatenate([jnp.broadcast_to(_rbf(jax.nn.sigmoid(ra)), (8, 1)),
                          jnp.broadcast_to(_rbf(jax.nn.sigmoid(rb_)), (8, 1))], axis=0)
    ys = [_rbf(_rbf(_dot(hid, wd_s[:, j * 128:(j + 1) * 128])) * rs) for j in range(NP)]

    for c in out_cps:
        c.wait()

    def patch(si, slot):
        g0 = mo((si // 16) * 16, 16)
        ww = mo(g0 // 2, 8)
        rows = g0 + 2 * lax.broadcasted_iota(I32, (8, 128), 0)
        for j in range(NP):
            ya, yb = ys[j][0:8, :], ys[j][8:16, :]
            hp = _unpk(h_s[j, pl.ds(ww, 8), :])
            xp = _unpk(x132[j, pl.ds(ww, 8), :])
            res = []
            for par in range(2):
                upd = jnp.where(rows + par == sa, ya, jnp.where(rows + par == sb, yb, 0.0))
                res.append(xp[par] + mod_s[5 * NP + j] * _rbf(hp[par] + upd))
            pst32[slot * 8:slot * 8 + 8, j * 128:(j + 1) * 128] = _pk(res[0], res[1])
        return pltpu.make_async_copy(pst_s.at[pl.ds(slot * 16, 16), :], out_hbm.at[pl.ds(g0, 16), :], sem_s.at[slot])

    ca = patch(sa, 0)
    cb = patch(sb, 1)
    ca.start()

    @pl.when(sa // 16 != sb // 16)
    def _():
        cb.start()
        cb.wait()

    ca.wait()


@jax.jit
def pallas_adaLN_cond__mha_block_cached__moe_arch_mod__prompt_kernel(
    A_x: jax.Array,
    A_k_cache: jax.Array,
    A_v_cache: jax.Array,
    A_wq: jax.Array,
    A_wo: jax.Array,
    B_x: jax.Array,
    B_w_r: jax.Array,
    B_w_gate: jax.Array,
    B_w_up: jax.Array,
    B_w_down: jax.Array,
    c: jax.Array,
    w_mod: jax.Array,
):
    del B_x
    hbm = pl.BlockSpec(memory_space=pl.ANY)
    dma = pltpu.SemaphoreType.DMA
    rq = pltpu.VMEM((5, 256, 128), I32)
    lo = pltpu.VMEM((5 * 16, R // 2, 128), I32)
    out = pl.pallas_call(
        _kernel,
        out_shape=jax.ShapeDtypeStruct((S, D), BF),
        in_specs=[hbm] * 11,
        out_specs=hbm,
        scratch_shapes=[
            pltpu.VMEM((NP, S, 128), BF),
            pltpu.VMEM((NP, S, 128), BF),
            pltpu.VMEM((NP, S, 128), BF),
            pltpu.VMEM((NSL * 7 * 4, R // 2, 128), I32),
            pltpu.VMEM((NP, S // 2, 128), I32),
            pltpu.VMEM((H, S // 2, 128), I32),
            pltpu.VMEM((H + 2, D, 128), BF),
            pltpu.VMEM((NP, H * DH, 128), BF),
            pltpu.VMEM((5 * 4, 1024, 128), I32),
            pltpu.VMEM((D, FF), BF),
            pltpu.VMEM((D, FF), BF),
            pltpu.VMEM((FF, D), BF),
            pltpu.VMEM((6 * NP, D, 128), BF),
            pltpu.VMEM((2, HPI, S, DH), BF),
            pltpu.VMEM((2, HPI, S, DH), BF),
            pltpu.VMEM((6 * NP, 8, 128), F32),
            pltpu.VMEM((NP, 2 * R, 128), F32),
            pltpu.VMEM((NP, 2 * R, 128), F32),
            lo, lo, rq, rq,
            pltpu.VMEM((1, D), BF),
            pltpu.VMEM((D,), BF),
            pltpu.VMEM((D, 128), F32),
            pltpu.VMEM((2, D // 2, 128), F32),
            pltpu.VMEM((2, D // 2, 128), F32),
            pltpu.VMEM((H + 2, 8, 128), F32),
            pltpu.VMEM((32, D), BF),
            dma((len(X_STAGES) - 1,)), dma((len(BLK) + H // IPI,)), dma((1,)), dma((1,)), dma((5,)),
            dma((2,)), dma((2,)), dma((1,)), dma((2,)),
        ],
        compiler_params=pltpu.CompilerParams(vmem_limit_bytes=124 * 1024 * 1024),
    )(A_x.reshape(S, D), A_k_cache.reshape(H, S, DH), A_v_cache.reshape(H, S, DH), A_wq, A_wo,
      B_w_r, B_w_gate, B_w_up, B_w_down, c, w_mod)
    return out.reshape(1, S, D)
```

```python
import jax
import jax.numpy as jnp
import jax.experimental.pallas as pl
import jax.experimental.pallas.tpu as pltpu
from jax import lax

BF = jnp.bfloat16
F32 = jnp.float32
I32 = jnp.int32

S = 2048
D = 1024
H = 32
DH = 128
FF = 3584
NP = D // 128
NF = FF // 128
EPS = 1e-5
QSCALE = float(DH ** -0.5 * 1.4426950408889634)
L_LO = 2.0 ** -30
L_HI = 2.0 ** 24

R = 64
NSL = S // (2 * R)
P0 = 8
IPI = 4
BQ = 256
HPI = 2
BLK = (0, 1, 2, 4, 6, 8)
LO_SPAN, LO_FIRST, LN_SPAN, LN_ST = 24, 12, 16, 3
X_STAGES = (0, 128, 384, 640, 1024, 2048)
DPI = 2

NN = (((1,), (0,)), ((), ()))
NT = (((1,), (1,)), ((), ()))


def _b16(x):
    return pltpu.bitcast(x, BF)


def _i32(x):
    return pltpu.bitcast(x, I32)


def _rbf(x):
    return x.astype(BF).astype(F32)


def _dot(a, b, dims=NN):
    return lax.dot_general(a, b, dims, preferred_element_type=F32)


def _unpk(w):
    return (pltpu.unpack_elementwise(w, index=0, packed_dtype=BF, unpacked_dtype=F32),
            pltpu.unpack_elementwise(w, index=1, packed_dtype=BF, unpacked_dtype=F32))


def _pk(even, odd):
    return pltpu.bitcast(pltpu.pack_elementwise([even, odd], packed_dtype=BF), I32)


def _zero_after(v):
    i = pltpu.bitcast(v[0:8, :], I32)
    return lax.shift_right_logical(lax.shift_right_logical(i, 31), 1)


def _tie(x, z):
    if z is None:
        return x
    return jnp.concatenate([x[r:r + 8] + z for r in range(0, x.shape[0], 8)], axis=0)


def _tief(x, z):
    return x if z is None else pltpu.bitcast(pltpu.bitcast(x, I32) + z[:, 0:1], F32)


def _ln_parts(parts, z1=None, z2=None):
    tot = parts[0]
    for p in parts[1:]:
        tot = tot + p
    m = _tief(jnp.sum(tot, axis=1, keepdims=True) * (1.0 / D), z1)
    dfs = [p - m for p in parts]
    sq = dfs[0] * dfs[0]
    for d in dfs[1:]:
        sq = sq + d * d
    v = _rbf(_rbf(jnp.sum(sq, axis=1, keepdims=True) * (1.0 / D)) + EPS)
    rs = lax.rsqrt(v)
    s = _rbf(v * rs)
    return dfs, _tief(rs * (2.0 - s * rs), z2)


def _strassen(prod):
    m1 = prod(0)
    m5 = prod(4)
    m4 = prod(3)
    m7 = prod(6)
    c11 = m1 + m4 - m5 + m7
    m3 = prod(2)
    c12 = m3 + m5
    m2 = prod(1)
    c21 = m2 + m4
    m6 = prod(5)
    c22 = m1 - m2 + m3 + m6
    return c11, c12, c21, c22


def _kernel(x_hbm, k_hbm, v_hbm, wq_hbm, wo_hbm, wr_hbm, wg_hbm, wu_hbm, wd_hbm, c_hbm, wm_hbm,
            out_hbm,
            x_s, x1_s, out_s, lq_s, h_s, q_s, wq_s, wo_s, ro_s, wg_s, wu_s, wd_s, wm_s, k_s, v_s, mod_s,
            t0_s, t1_s, lo0_s, lo1_s, re_s, rf_s, c_s, wr_s, ccol_s, cc2_s, cs2_s, b_s, pst_s,
            sem_x, sem_wq, sem_wo, sem_mlp, sem_m, sem_k, sem_v, sem_o, sem_s):
    wq32 = wq_s.bitcast(I32)
    wo32 = wo_s.bitcast(I32)
    wm32 = wm_s.bitcast(I32)
    k32 = k_s.bitcast(I32)
    v32 = v_s.bitcast(I32)
    x32 = x_s.bitcast(I32)
    x132 = x1_s.bitcast(I32)
    out32 = out_s.bitcast(I32)
    pst32 = pst_s.bitcast(I32)

    def mo(i, m):
        return i if isinstance(i, int) else pl.multiple_of(i, m)

    def col(j):
        return pl.ds(mo(j * 128, 128), 128)

    def cp_x(st, j):
        r0, n = X_STAGES[st], X_STAGES[st + 1] - X_STAGES[st]
        return pltpu.make_async_copy(x_hbm.at[pl.ds(r0, n), col(j)], x_s.at[j, pl.ds(r0, n), :], sem_x.at[st])

    def cp_wq(h, g):
        src = h if not isinstance(h, int) or h < H else h - 2
        return pltpu.make_async_copy(wq_hbm.at[:, col(src)], wq_s.at[h], sem_wq.at[g])

    def item(i):
        if isinstance(i, int):
            return (i, NSL // 2) if i < P0 else (P0 + (i - P0) // 2, (i - P0) % 2 * (NSL // 2))
        j = jnp.maximum(i - P0, 0)
        return (jnp.where(i < P0, i, P0 + j // 2), jnp.where(i < P0, NSL // 2, j % 2 * (NSL // 2)))

    NPAIR = H // 2
    NB = (P0 + 2 * (NPAIR - P0)) // IPI
    G_LOOP = P0 // IPI

    NBLK = len(BLK) - 1

    def wq_group(h):
        p = h // 2
        if p < P0:
            return 0 if p == 0 else min(k for k in range(1, NBLK) if p <= BLK[k + 1])
        return NBLK if p == P0 else NBLK + 1 + (p - P0 - 1) // (IPI // 2)

    def cp_m(j, g):
        return pltpu.make_async_copy(wm_hbm.at[:, col(j)], wm_s.at[j], sem_m.at[g])

    def m_panel(i):
        return NP + i // 2 + 4 * (i % 2)

    def cp_wo(j):
        return pltpu.make_async_copy(wo_hbm.at[:, col(j)], wo_s.at[j], sem_wo.at[0])

    NG = H // HPI

    def cp_mlp(g):
        return [pltpu.make_async_copy(src.at[pl.ds(mo(g * n, 16), n), :], dst.at[pl.ds(mo(g * n, 16), n), :], sem_mlp.at[0])
                for src, dst, n in ((wg_hbm, wg_s, D // NG), (wu_hbm, wu_s, D // NG), (wd_hbm, wd_s, FF // NG))]

    def cp_kv(g, slot):
        return (pltpu.make_async_copy(k_hbm.at[pl.ds(mo(g * HPI, HPI), HPI)], k_s.at[slot], sem_k.at[slot]),
                pltpu.make_async_copy(v_hbm.at[pl.ds(mo(g * HPI, HPI), HPI)], v_s.at[slot], sem_v.at[slot]))

    def cp_o(r0, n, j, i):
        return pltpu.make_async_copy(out_s.at[j, pl.ds(r0, n), :], out_hbm.at[pl.ds(r0, n), col(j)], sem_o.at[i])

    cp_c = pltpu.make_async_copy(c_hbm, c_s, sem_s.at[0])
    cp_r = pltpu.make_async_copy(wr_hbm, wr_s, sem_s.at[1])
    cp_c.start()

    @pl.loop(0, 2)
    def _(h):
        cp_wq(h, 0).start()

    @pl.loop(0, NP)
    def _(i):
        cp_m(m_panel(i), i // 2).start()

    for st in range(4):
        @pl.loop(0, NP)
        def _(j):
            cp_x(st, j).start()

    for k in (1, 2):
        hs = [h for h in range(H + 2) if wq_group(h) == k]

        @pl.loop(hs[0], hs[-1] + 1)
        def _(h):
            cp_wq(h, k).start()

    @pl.loop(0, NP)
    def _(j):
        cp_x(4, j).start()

    bst = {}

    def rq_step(p, dst, r0, z=None, bias=False):
        a, b = 2 * p, 2 * p + 1

        def ld(h, half):
            return _unpk(_tie(wq32[h, pl.ds(half * 256 + r0, 32), :], z))
        b11, b12, b21, b22 = ld(a, 0), ld(b, 0), ld(a, 1), ld(b, 1)
        for i, (u, v, sg) in enumerate(((b11, b22, 1), (b12, b22, -1), (b21, b11, -1), (b11, b12, 1), (b21, b22, 1))):
            dst[i, r0:r0 + 32, :] = _pk(u[0] + v[0], u[1] + v[1]) if sg > 0 else _pk(u[0] - v[0], u[1] - v[1])
        if bias:
            sh = [cs2_s[par, half * 256 + r0:half * 256 + r0 + 32, :] for half in range(2) for par in range(2)]
            for h, up, dn in ((a, b11, b21), (b, b12, b22)):
                t = up[0] * sh[0] + up[1] * sh[1] + dn[0] * sh[2] + dn[1] * sh[3]
                t = (t[0:8] + t[8:16]) + (t[16:24] + t[24:32])
                bst[h is a] = t if r0 == 0 else bst[h is a] + t
                if r0 == 224:
                    b_s[h] = jnp.broadcast_to(jnp.sum(bst[h is a], axis=0, keepdims=True), (8, 128))

    def rq_combos(p, dst):
        for r0 in range(0, 256, 32):
            rq_step(p, dst, r0)

    def load_q(h, w0, nw):
        e, o = _unpk(q_s[h, pl.ds(w0, nw), :])
        b = jnp.concatenate([b_s[h]] * (nw // 8), axis=0)
        return _b16(_pk(e + b, o + b))

    def lq_store(s, kc, hs, w0, nw):
        ops = [(a11 + a22, a21 + a22, a11, a22, a11 + a12, a21 - a11, a12 - a22) for a11, a12, a21, a22 in hs]
        for i in range(7):
            lq_s[(s * 7 + i) * 4 + kc, w0:w0 + nw, :] = _pk(ops[0][i], ops[1][i])

    def ln1(s, w0, nw, z, z1, z2):
        hs = [[], []]
        for half in range(2):
            ww = s * R + half * (R // 2) + w0
            xs = [_unpk(_tie(x32[j, ww:ww + nw, :], z)) for j in range(NP)]
            for par in range(2):
                ds, inv = _ln_parts([x_[par] for x_ in xs], z1, z2)
                hs[par].append([(ds[j] * inv) * mod_s[NP + j, 0:1, :] for j in range(NP)])
        for kc in range(4):
            lq_store(s, kc, [(hs[par][0][kc], hs[par][0][kc + 4], hs[par][1][kc], hs[par][1][kc + 4])
                             for par in range(2)], w0, nw)

    def q_slab(p, rsrc, s):
        a, b = 2 * p, 2 * p + 1
        toks = []

        def prod(i):
            lhs = jnp.concatenate([_b16(lq_s[(s * 7 + i) * 4 + kc]) for kc in range(4)], axis=1)
            if i == 1:
                w = wq32[a, 0:256, :]
            elif i == 4:
                w = wq32[b, 256:512, :]
            else:
                w = rsrc[{0: 0, 2: 1, 3: 2, 5: 3, 6: 4}[i]]
            m = _dot(lhs, _b16(w))
            toks.append(m)
            return m

        c11, c12, c21, c22 = _strassen(prod)
        w0 = mo(s * R, R)
        q_s[a, pl.ds(w0, R // 2), :] = _i32(c11.astype(BF))
        q_s[b, pl.ds(w0, R // 2), :] = _i32(c12.astype(BF))
        q_s[a, pl.ds(w0 + R // 2, R // 2), :] = _i32(c21.astype(BF))
        q_s[b, pl.ds(w0 + R // 2, R // 2), :] = _i32(c22.astype(BF))
        return toks

    cp_c.wait()
    cf = c_s[...].astype(F32)
    sc = _rbf(cf * _rbf(jax.nn.sigmoid(cf)))
    sc16 = jnp.broadcast_to(sc, (16, D)).astype(BF)
    scb = jnp.broadcast_to(sc, (128, D))
    for j in range(NP):
        ccol_s[j * 128:(j + 1) * 128, :] = scb[:, j * 128:(j + 1) * 128].T
    ce_s, co_s = cc2_s.at[0], cc2_s.at[1]
    ce_s[...] = ccol_s[pl.ds(0, D // 2, stride=2), :]
    co_s[...] = ccol_s[pl.ds(1, D // 2, stride=2), :]

    for h in range(2):
        cp_wq(h, 0).wait()
    rp = (re_s, rf_s)
    rq_combos(0, rp[0])

    for g in range(4):
        for i in range(2):
            cp_m(m_panel(2 * g + i), g).wait()
        for j in (g, g + 4):
            mod_s[NP + j] = _rbf(1.0 + _rbf(_dot(sc16, _b16(wm32[NP + j]))[0:8, :])) * QSCALE

    npc = R // 16

    def ln1_spread(slabs, toks):
        n = len(slabs) * npc
        for i in range(n):
            zs = [_zero_after(toks[int((i + d) * (len(toks) - 1) / (n + 2))]) if toks else None for d in (0.0, 1.0, 2.0)]
            ln1(slabs[i // npc], i % npc * 8, 8, *zs)

    for st in range(4):
        for j in range(NP):
            cp_x(st, j).wait()
        slabs = lambda i: tuple(range(X_STAGES[i] // (2 * R), X_STAGES[i + 1] // (2 * R)))
        for s in slabs(st - 1) if st else ():
            q_slab(0, rp[0], s)
        ln1_spread(slabs(st), [])

    for k in range(1, NBLK):
        toks = []
        for h in range(2 * NPAIR):
            if wq_group(h) == k:
                cp_wq(h, k).wait()
        if k == NBLK - 2:
            for j in range(NP):
                cp_x(4, j).wait()
        if k == NBLK - 1:
            for j in range(NP):
                cp_m(j, 4).wait()
            for j in range(NP):
                sa = _rbf(_dot(sc16, _b16(wm32[j]))[0:1, :]) * QSCALE
                ccol_s[j * 128:(j + 1) * 128, :] = jnp.broadcast_to(sa, (128, 128)).T
            for par in range(2):
                cs2_s[par] = ccol_s[pl.ds(par, D // 2, stride=2), :]
        if k == 1:
            for s in slabs(3):
                q_slab(0, rp[0], s)
            rq_combos(1, rp[1])
        for p in range(BLK[k], BLK[k + 1]):
            for s in range(NSL // 2):
                tk = q_slab(p, rp[p % 2], s)
                toks += tk
                rq_step(p + 1 if p + 1 < P0 else item(0)[0], rp[(p + 1) % 2], s * 32, _zero_after(tk[0]),
                        bias=p + 1 == P0)
            if p == BLK[k]:
                if k == 2:
                    for j in range(NP):
                        cp_m(j, 4).start()
                for h in range(6, H + 2):
                    if (None, 3 <= wq_group(h) < NBLK, False, wq_group(h) == NBLK, wq_group(h) > NBLK)[k]:
                        cp_wq(h, wq_group(h)).start()
        if k >= NBLK - 2:
            s0 = NSL // 4 * (k - NBLK + 4)
            ln1_spread(tuple(range(s0, s0 + NSL // 4)), toks)

    for h in (2 * P0, 2 * P0 + 1):
        cp_wq(h, NBLK).wait()
    cp_r.start()

    def phase_b(g, carry):
        @pl.when(g >= G_LOOP)
        def _():
            for h in range(IPI):
                cp_wq(2 * P0 + 2 + (g - G_LOOP) * IPI + h, NBLK + 1 + g - G_LOOP).wait()

        @pl.when(g == 0)
        def _():
            for c in cp_kv(0, 0):
                c.start()
            for j in range(NP):
                cp_wo(j).start()
            for j in range(2 * NP, 6 * NP):
                cp_m(j, 4).start()

        for u in range(IPI):
            p, s0 = item(g * IPI + u)
            pn, _ = item(g * IPI + u + 1)
            for s in range(NSL // 2):
                toks = q_slab(p, rp[(P0 + u) % 2], s0 + s)
                for i in range(-(-4 * s // 3), -(-4 * (s + 1) // 3)):
                    if i < 8:
                        rq_step(pn, rp[(P0 + u + 1) % 2], i * 32, _zero_after(toks[3 * (i % 2)]), bias=True)
        return carry

    lax.fori_loop(0, NB, phase_b, 0)

    for j in range(NP):
        cp_wo(j).wait()

    for j in range(2 * NP, 6 * NP):
        cp_m(j, 4).wait()

    def ro_job(g, n, r0, z):
        w0 = mo(g * 64, 64)

        def ld(j, half):
            return _unpk(_tie(wo32[j, pl.ds(w0 + half * 1024 + r0, 16), :], z))
        b11, b12, b21, b22 = ld(n, 0), ld(n + 4, 0), ld(n, 1), ld(n + 4, 1)
        for i, (u, v, sg) in enumerate(((b11, b22, 1), (b12, b22, -1), (b21, b11, -1), (b11, b12, 1), (b21, b22, 1))):
            ro_s[i * 4 + n, pl.ds(w0 + r0, 16), :] = (_pk(u[0] + v[0], u[1] + v[1]) if sg > 0
                                                     else _pk(u[0] - v[0], u[1] - v[1]))

    mst = {}

    def mod_job(j, r, z):
        we, wo_ = _unpk(_tie(wm32[j, r:r + 64, :], z))
        t = we * ce_s[r:r + 64, :] + wo_ * co_s[r:r + 64, :]
        t = jnp.sum(t.reshape(8, 8, 128), axis=0)
        mst['acc'] = t if r == 0 else mst['acc'] + t
        if r == 448:
            v = _rbf(jnp.sum(mst['acc'], axis=0, keepdims=True))
            v = jnp.where(j // NP == 4, _rbf(1.0 + v), v)
            mod_s[j] = jnp.broadcast_to(v, (8, 128))

    def lo_combos(w0, r, dst, g, z):
        def ld(h, half):
            return _unpk(_tie(q_s[h, pl.ds(mo(w0 + half * (r // 2), r // 2), r // 2), :], z))
        a11, a12, a21, a22 = ld(g, 0), ld(g + 16, 0), ld(g, 1), ld(g + 16, 1)
        for i, (u, v, sg) in enumerate(((a11, a22, 1), (a21, a22, 1), (a11, a12, 1), (a21, a11, -1), (a12, a22, -1))):
            dst[i * 16 + g, 0:r // 2, :] = (_pk(u[0] + v[0], u[1] + v[1]) if sg > 0
                                            else _pk(u[0] - v[0], u[1] - v[1]))

    def attn_group(g, carry):
        lmin = jnp.full((8, 1), L_HI, F32)
        lmax = jnp.full((8, 1), L_LO, F32)
        slot = g % 2
        for c in cp_kv(g, slot):
            c.wait()
        ja = [lambda z, u=u, n=n, r0=r0: ro_job(g * (16 // NG) + u, n, r0, z)
              for u in range(16 // NG) for n in range(4) for r0 in range(0, 64, 16)]
        jb = [lambda z, jj=jj, r=r: mod_job(2 * NP + HPI * g + jj, r, z) for jj in range(HPI) for r in range(0, 512, 64)]
        jobs = [x for pair in zip(ja, jb) for x in pair]
        nch = HPI * (S // BQ)
        ntok = (nch - 1) * 4
        tc = 0
        for hh in range(HPI):
            h = g * HPI + hh
            k = _b16(k32[slot, hh])
            v = _b16(v32[slot, hh])
            for ci in range(S // BQ):
                q = load_q(h, ci * BQ // 2, BQ // 2)
                s = _dot(q, k, NT)
                if hh == 0 and ci == 0:
                    for c in cp_kv((g + 1) % NG, 1 - slot):
                        c.start()
                    for c in cp_mlp(g):
                        c.start()
                for tt in range(4):
                    z = _zero_after(s[0:8, tt * 512:tt * 512 + 128])
                    todo = jobs[tc * len(jobs) // ntok:(tc + 1) * len(jobs) // ntok]
                    for f in todo:
                        f(z)
                    tc += 1
                p = jnp.exp2(s)
                l = jnp.sum(p, axis=1, keepdims=True)
                r0_ = pl.reciprocal(l, approx=True)
                o = _dot(p.astype(BF), v) * (r0_ * (2.0 - l * r0_))
                q_s[h, pl.ds(ci * BQ // 2, BQ // 2), :] = _i32(o.astype(BF))
                for t in range(BQ // 8):
                    lt = l[t * 8:(t + 1) * 8]
                    lmin = jnp.minimum(lmin, lt)
                    lmax = jnp.maximum(lmax, lt)
        ok = jnp.logical_and(lmin >= L_LO, lmax <= L_HI)
        return jnp.maximum(carry, jnp.max(jnp.where(ok, 0, 1)))

    bad = lax.fori_loop(0, NG, attn_group, jnp.int32(0)) > 0

    def safe_attention():
        def safe_pair(p, carry):
            rq_combos(p, re_s)

            def qs(s, c2):
                q_slab(p, re_s, s)
                return c2

            lax.fori_loop(0, NSL, qs, 0)

            def one_head(hh, c2):
                h = 2 * p + hh
                ck = pltpu.make_async_copy(k_hbm.at[h], k_s.at[1, 0], sem_k.at[1])
                cv = pltpu.make_async_copy(v_hbm.at[h], v_s.at[1, 0], sem_v.at[1])
                ck.start()
                cv.start()
                ck.wait()
                cv.wait()

                def chunk(ci, c3):
                    w0 = mo(ci * 64, 64)
                    q = load_q(h, w0, 64)
                    s = _dot(q, _b16(k32[1, 0]), NT)
                    p_ = jnp.exp2(s - jnp.max(s, axis=1, keepdims=True))
                    l = jnp.sum(p_, axis=1, keepdims=True)
                    o = _dot(p_.astype(BF), _b16(v32[1, 0])) * (1.0 / l)
                    q_s[h, pl.ds(w0, 64), :] = _i32(o.astype(BF))
                    return c3

                lax.fori_loop(0, S // 128, chunk, 0)
                return c2

            lax.fori_loop(0, 2, one_head, 0)
            return carry

        lax.fori_loop(0, NPAIR, safe_pair, 0)

    pl.when(bad)(safe_attention)

    cp_r.wait()
    wr = wr_s[...].astype(F32).reshape(1, D)
    cw = [mod_s[4 * NP + j, 0:1, :] * wr[:, j * 128:(j + 1) * 128] for j in range(NP)]
    sw = mod_s[3 * NP, 0:1, :] * wr[:, 0:128]
    for j in range(1, NP):
        sw = sw + mod_s[3 * NP + j, 0:1, :] * wr[:, j * 128:(j + 1) * 128]
    sw = jnp.sum(sw, axis=1, keepdims=True)

    def o_slab(w0, r, lsrc, t_ref, side, split=False, first=False):
        cnt = [0]
        prods = []
        for n in range(4):
            def prod(i, n=n):
                if i == 2:
                    pan = [q_s[g, pl.ds(mo(w0, r // 2), r // 2), :] for g in range(16)]
                elif i == 3:
                    pan = [q_s[g + 16, pl.ds(mo(w0 + r // 2, r // 2), r // 2), :] for g in range(16)]
                else:
                    li = {0: 0, 1: 1, 4: 2, 5: 3, 6: 4}[i]
                    pan = [lsrc[li * 16 + g, 0:r // 2, :] for g in range(16)]
                lhs = jnp.concatenate([_b16(a) for a in pan], axis=1)
                if i == 1:
                    w = wo32[n, 0:1024, :]
                elif i == 4:
                    w = wo32[n + 4, 1024:2048, :]
                else:
                    w = ro_s[{0: 0, 2: 1, 3: 2, 5: 3, 6: 4}[i] * 4 + n]
                m = _dot(lhs, _b16(w))
                side(cnt[0], m)
                cnt[0] += 1
                return m
            prods.append(prod)
        if first:
            for n in range(4):
                t_ref[n, r:2 * r, :] = prods[n](3)
                t_ref[n + 4, 0:r, :] = prods[n](2)
            for n in range(4):
                m1, m5, m2 = prods[n](0), prods[n](4), prods[n](1)
                m4, m3 = t_ref[n, r:2 * r, :], t_ref[n + 4, 0:r, :]
                t_ref[n, 0:r, :] = m1 + m4 - m5 + prods[n](6)
                t_ref[n + 4, 0:r, :] = m3 + m5
                t_ref[n, r:2 * r, :] = m2 + m4
                t_ref[n + 4, r:2 * r, :] = m1 - m2 + m3 + prods[n](5)
            return
        for n in range(4):
            prod = prods[n]
            if split:
                m1, m5, m4, m7, m3 = prod(0), prod(4), prod(3), prod(6), prod(2)
                c11, c12, c21, c22 = m1 + m4 - m5 + m7, m3 + m5, m4, m1 + m3
            else:
                c11, c12, c21, c22 = _strassen(prod)
            t_ref[n, 0:r, :] = c11
            t_ref[n + 4, 0:r, :] = c12
            t_ref[n, r:2 * r, :] = c21
            t_ref[n + 4, r:2 * r, :] = c22
        if split:
            for n in range(4):
                m2, m6 = prods[n](1), prods[n](5)
                t_ref[n, r:2 * r, :] = t_ref[n, r:2 * r, :] + m2
                t_ref[n + 4, r:2 * r, :] = t_ref[n + 4, r:2 * r, :] + (m6 - m2)

    state = {}

    def ln2(rr, t_ref, p0, z, z1=None, z2=None):
        m1, i1, m2, i2 = state['top']
        ww = mo(rr // 2, 8)
        x1 = [[], []]
        for j in range(NP):
            xe, xo = _unpk(_tie(x32[j, pl.ds(ww, 8), :], z))
            ga = mod_s[2 * NP + j]
            e = xe + t_ref[j, pl.ds(p0, 8, stride=2), :] * ga
            o = xo + t_ref[j, pl.ds(p0 + 1, 8, stride=2), :] * ga
            x132[j, pl.ds(ww, 8), :] = _pk(e, o)
            x1[0].append(e)
            x1[1].append(o)
        hs, os_ = [], []
        for par in range(2):
            ds, inv = _ln_parts(x1[par], z1, z2)
            rd = ds[0] * cw[0]
            for j in range(1, NP):
                rd = rd + ds[j] * cw[j]
            v = _rbf(jnp.sum(rd, axis=1, keepdims=True) * inv + sw)
            hj = [(ds[j] * inv) * mod_s[4 * NP + j] + mod_s[3 * NP + j] for j in range(NP)]
            hs.append(hj)
            os_.append([x1[par][j] + mod_s[5 * NP + j] * hj[j] for j in range(NP)])
            idx = 2 * sub + (rr + par)
            gt1 = v > m1
            gt2 = v > m2
            m2 = jnp.where(gt1, m1, jnp.where(gt2, v, m2))
            i2 = jnp.where(gt1, i1, jnp.where(gt2, idx, i2))
            m1 = jnp.where(gt1, v, m1)
            i1 = jnp.where(gt1, idx, i1)
        for j in range(NP):
            h_s[j, pl.ds(ww, 8), :] = _pk(hs[0][j], hs[1][j])
            out32[j, pl.ds(ww, 8), :] = _pk(os_[0][j], os_[1][j])
        state['top'] = (m1, i1, m2, i2)

    ninf = jnp.full((8, 128), -jnp.inf, F32)
    sub = lax.broadcasted_iota(I32, (8, 128), 0)
    tb = (t0_s, t1_s)
    lb = (lo0_s, lo1_s)

    def d_step(row, r, slot, r_next, r_prev, split=False, first=False):
        jobs = []
        if r_next:
            g0 = LO_FIRST if first else 0
            for g in range(16):
                jobs.append(((g0 + g * (LO_SPAN if not first else 27 - g0) // 16,),
                             lambda z, g=g: lo_combos((row + 2 * r) // 2, r_next, lb[1 - slot], g, z)))
        if r_prev:
            npc = 2 * r_prev // 16
            for i in range(npc):
                k = (LO_FIRST if first else 0) + i * (LN_SPAN // 2 if first else LN_SPAN) // npc
                jobs.append(((k, k + LN_ST, k + 2 * LN_ST),
                             lambda *z, i=i: ln2(row - 2 * r_prev + i * 16, tb[1 - slot], i * 16, *z)))
        if split:
            for i in range(r // 16):
                jobs.append(((20 + 2 * i, 21 + 2 * i, 22 + 2 * i),
                             lambda *z, i=i: ln2(row + i * 16, tb[slot], i * 16, *z)))
        zs = []

        def side(k, m):
            zs.append(_zero_after(m) if any(k in ks for ks, _ in jobs) else None)
            for ks, f in jobs:
                if ks[-1] == k:
                    f(*[zs[i] for i in ks])

        o_slab(row // 2, r, lb[slot], tb[slot], side, split, first)

    ND = (NSL - 2) // DPI
    OB = 4 * R
    last = (NSL - 1) * 2 * R

    def d_loop(i, top):
        state['top'] = top
        row = mo(2 * R + i * DPI * 2 * R, 2 * R)
        for u in range(DPI):
            d_step(row + u * 2 * R, R, (u + 1) % 2, R, R)
            if u % 2 == 1:
                for j in range(NP):
                    cp_o(mo(row + (u - 2) * 2 * R, OB), OB, j, 0).start()
        return state['top']

    state['top'] = (ninf, sub + S, ninf, sub + S + 8)
    for g in range(16):
        lo_combos(0, R, lb[0], g, None)
    d_step(0, R, 0, R, 0, first=True)
    if ND == 1:
        d_loop(0, state['top'])
    else:
        state['top'] = lax.fori_loop(0, ND, d_loop, state['top'])
    for g in range(16):
        lo_combos(last // 2, R // 2, lb[1], g, None)
    d_step(last, R // 2, 1, R // 2, R, first=True)
    d_step(last + R, R // 2, 0, 0, R // 2, split=True)
    for i in range(R // 32, R // 16):
        ln2(last + R + i * 16, tb[0], i * 16, None)
    out_cps = [cp_o(i * OB, OB, j, 0) for i in range((NSL - 2) // 2) for j in range(NP)]
    for j in range(NP):
        c = cp_o(last - 2 * R, 4 * R, j, 0)
        c.start()
        out_cps.append(c)
    m1, i1, m2, i2 = state['top']

    big = jnp.int32(1 << 30)
    ra = jnp.max(m1, axis=0, keepdims=True)
    ia = jnp.min(jnp.where(m1 == ra, i1, big), axis=0, keepdims=True)
    win = i1 == ia
    mm = jnp.where(win, m2, m1)
    ii = jnp.where(win, i2, i1)
    rb_ = jnp.max(mm, axis=0, keepdims=True)
    ib = jnp.min(jnp.where(mm == rb_, ii, big), axis=0, keepdims=True)
    sa = jnp.clip(ia[0, 0], 0, S - 1)
    sb = jnp.clip(ib[0, 0], 0, S - 1)

    def hrow(si, j):
        e, o = _unpk(jnp.broadcast_to(h_s[j, pl.ds(si // 2, 1), :], (8, 128)))
        return jnp.where(si % 2 == 0, e, o)

    xs = jnp.concatenate([jnp.concatenate([hrow(si, j) for j in range(NP)], axis=1) for si in (sa, sb)],
                         axis=0).astype(BF)

    for g in range(NG):
        for c in cp_mlp(g):
            c.wait()
    for c in cp_kv(0, NG % 2):
        c.wait()
    hid = []
    for j in range(NF):
        g = _rbf(_dot(xs, wg_s[:, j * 128:(j + 1) * 128]))
        u = _rbf(_dot(xs, wu_s[:, j * 128:(j + 1) * 128]))
        g = _rbf(g * _rbf(jax.nn.sigmoid(g)))
        hid.append((g * u).astype(BF))
    hid = jnp.concatenate(hid, axis=1)
    rs = jnp.concatenate([jnp.broadcast_to(_rbf(jax.nn.sigmoid(ra)), (8, 128)),
                          jnp.broadcast_to(_rbf(jax.nn.sigmoid(rb_)), (8, 128))], axis=0)
    ys = [_rbf(_rbf(_dot(hid, wd_s[:, j * 128:(j + 1) * 128])) * rs) for j in range(NP)]

    for c in out_cps:
        c.wait()

    def patch(si, slot):
        g0 = mo((si // 16) * 16, 16)
        ww = mo(g0 // 2, 8)
        rows = g0 + 2 * lax.broadcasted_iota(I32, (8, 128), 0)
        for j in range(NP):
            ya, yb = ys[j][0:8, :], ys[j][8:16, :]
            hp = _unpk(h_s[j, pl.ds(ww, 8), :])
            xp = _unpk(x132[j, pl.ds(ww, 8), :])
            res = []
            for par in range(2):
                upd = jnp.where(rows + par == sa, ya, jnp.where(rows + par == sb, yb, 0.0))
                res.append(xp[par] + mod_s[5 * NP + j] * _rbf(hp[par] + upd))
            pst32[slot * 8:slot * 8 + 8, j * 128:(j + 1) * 128] = _pk(res[0], res[1])
        return pltpu.make_async_copy(pst_s.at[pl.ds(slot * 16, 16), :], out_hbm.at[pl.ds(g0, 16), :], sem_s.at[slot])

    ca = patch(sa, 0)
    cb = patch(sb, 1)
    ca.start()

    @pl.when(sa // 16 != sb // 16)
    def _():
        cb.start()
        cb.wait()

    ca.wait()


@jax.jit
def pallas_adaLN_cond__mha_block_cached__moe_arch_mod__prompt_kernel(
    A_x: jax.Array,
    A_k_cache: jax.Array,
    A_v_cache: jax.Array,
    A_wq: jax.Array,
    A_wo: jax.Array,
    B_x: jax.Array,
    B_w_r: jax.Array,
    B_w_gate: jax.Array,
    B_w_up: jax.Array,
    B_w_down: jax.Array,
    c: jax.Array,
    w_mod: jax.Array,
):
    del B_x
    hbm = pl.BlockSpec(memory_space=pl.ANY)
    dma = pltpu.SemaphoreType.DMA
    rq = pltpu.VMEM((5, 256, 128), I32)
    lo = pltpu.VMEM((5 * 16, R // 2, 128), I32)
    out = pl.pallas_call(
        _kernel,
        out_shape=jax.ShapeDtypeStruct((S, D), BF),
        in_specs=[hbm] * 11,
        out_specs=hbm,
        scratch_shapes=[
            pltpu.VMEM((NP, S, 128), BF),
            pltpu.VMEM((NP, S, 128), BF),
            pltpu.VMEM((NP, S, 128), BF),
            pltpu.VMEM((NSL * 7 * 4, R // 2, 128), I32),
            pltpu.VMEM((NP, S // 2, 128), I32),
            pltpu.VMEM((H, S // 2, 128), I32),
            pltpu.VMEM((H + 2, D, 128), BF),
            pltpu.VMEM((NP, H * DH, 128), BF),
            pltpu.VMEM((5 * 4, 1024, 128), I32),
            pltpu.VMEM((D, FF), BF),
            pltpu.VMEM((D, FF), BF),
            pltpu.VMEM((FF, D), BF),
            pltpu.VMEM((6 * NP, D, 128), BF),
            pltpu.VMEM((2, HPI, S, DH), BF),
            pltpu.VMEM((2, HPI, S, DH), BF),
            pltpu.VMEM((6 * NP, 8, 128), F32),
            pltpu.VMEM((NP, 2 * R, 128), F32),
            pltpu.VMEM((NP, 2 * R, 128), F32),
            lo, lo, rq, rq,
            pltpu.VMEM((1, D), BF),
            pltpu.VMEM((D,), BF),
            pltpu.VMEM((D, 128), F32),
            pltpu.VMEM((2, D // 2, 128), F32),
            pltpu.VMEM((2, D // 2, 128), F32),
            pltpu.VMEM((H + 2, 8, 128), F32),
            pltpu.VMEM((32, D), BF),
            dma((len(X_STAGES) - 1,)), dma((len(BLK) + H // IPI,)), dma((1,)), dma((1,)), dma((5,)),
            dma((2,)), dma((2,)), dma((1,)), dma((2,)),
        ],
        compiler_params=pltpu.CompilerParams(vmem_limit_bytes=124 * 1024 * 1024),
    )(A_x.reshape(S, D), A_k_cache.reshape(H, S, DH), A_v_cache.reshape(H, S, DH), A_wq, A_wo,
      B_w_r, B_w_gate, B_w_up, B_w_down, c, w_mod)
    return out.reshape(1, S, D)
```
